```python
import jax
import jax.numpy as jnp

def _softmax(x, axis=-1):
    return jax.nn.softmax(x, axis=axis)
def _gelu(x):
    return jax.nn.gelu(x, approximate=True)
def _silu(x):
    return jax.nn.silu(x)
def _sigmoid(x):
    return jax.nn.sigmoid(x)
def _layernorm(x, axis=-1, eps=1e-5):
    m = jnp.mean(x, axis=axis, keepdims=True)
    v = jnp.var(x, axis=axis, keepdims=True)
    return (x - m) / jnp.sqrt(v + eps)
def _scatter_add(tgt, idx, src, axis=0):
    return tgt.at[idx].add(src)
def _segment_sum(src, seg, n):
    return jax.ops.segment_sum(src, seg, n)
class _Rng:
    def __init__(self, key):
        self._k = key
    def _next(self):
        self._k, sub = jax.random.split(self._k)
        return sub
    def normal(self, shape):
        return jax.random.normal(self._next(), shape, dtype=jnp.bfloat16)
    def randint(self, lo, hi, shape):
        return jax.random.randint(self._next(), shape, lo, hi, dtype=jnp.int32)
    def uniform(self, shape, lo=0.0, hi=1.0):
        return jax.random.uniform(self._next(), shape, jnp.bfloat16, lo, hi)
    def permutation(self, n):
        return jax.random.permutation(self._next(), n)


kernel_name = 'recurrent_scan__compressed_kv_cla__dense_activation_gelu__decode'

def setup_inputs():
    _rng = _Rng(jax.random.key(int.from_bytes(__import__("os").urandom(4), "little")))
    _w = (lambda a: (lambda t: t.astype(jnp.bfloat16) if jnp.issubdtype(t.dtype, jnp.floating) else t)(jnp.asarray(a)))
    def _A_setup():
        B, H, Sq, Sk, D, M = 2, 32, 1, 16384, 128, 512
        Dc = 4 * D
        return {
            "x": _w((lambda *s: _rng.normal(s) * 0.05)(B, Sq, M)),
            "c_kv": _w((lambda *s: _rng.normal(s) * 0.05)(B, Sk, Dc)),
            "w_q": _w((lambda *s: _rng.normal(s) * 0.05)(M, H, D) * (M ** -0.5)),
            "w_uk": _w((lambda *s: _rng.normal(s) * 0.05)(Dc, H, D) * (Dc ** -0.5)),
            "w_uv": _w((lambda *s: _rng.normal(s) * 0.05)(Dc, H, D) * (Dc ** -0.5)),
            "w_o": _w((lambda *s: _rng.normal(s) * 0.05)(H, D, M) * ((H * D) ** -0.5)),
        }
    _A_in = _A_setup()

    def _B_setup():
        B, S, D, F = 2, 1, 512, 1792
        return {
            "x": _w((lambda *s: _rng.normal(s) * 0.05)(B, S, D)),
            "w1": _w((lambda *s: _rng.normal(s) * 0.05)(D, F) * (D ** -0.5)),
            "b1": _w((lambda *s: _rng.normal(s) * 0.05)(F) * 0.01),
            "w2": _w((lambda *s: _rng.normal(s) * 0.05)(F, D) * (F ** -0.5)),
            "b2": _w((lambda *s: _rng.normal(s) * 0.05)(D) * 0.01),
        }
    _B_in = _B_setup()

    return {
        "A_x": _A_in["x"],
        "A_c_kv": _A_in["c_kv"],
        "A_w_q": _A_in["w_q"],
        "A_w_uk": _A_in["w_uk"],
        "A_w_uv": _A_in["w_uv"],
        "A_w_o": _A_in["w_o"],
        "B_x": _B_in["x"],
        "B_w1": _B_in["w1"],
        "B_b1": _B_in["b1"],
        "B_w2": _B_in["w2"],
        "B_b2": _B_in["b2"],
    }

def reference(A_x, A_c_kv, A_w_q, A_w_uk, A_w_uv, A_w_o, B_x, B_w1, B_b1, B_w2, B_b2):
    def _A_ref(x, c_kv, w_q, w_uk, w_uv, w_o):
        B, Sq, M = x.shape[0], x.shape[1], x.shape[2]
        Sk = c_kv.shape[1]
        H, D = w_q.shape[1], w_q.shape[2]
        q = jnp.einsum("bqm,mhd->bhqd", x, w_q)
        k = jnp.einsum("bkc,chd->bhkd", c_kv, w_uk)
        v = jnp.einsum("bkc,chd->bhkd", c_kv, w_uv)
        scores = jnp.einsum("bhqd,bhkd->bhqk", q, k) * (D ** -0.5)
        off = Sk - Sq
        qi = jnp.arange(Sq)[:, None]
        kj = jnp.arange(Sk)[None, :]
        cmask = kj <= (qi + off)
        scores = jnp.where(cmask[None, None], scores, -1e9)
        p = _softmax(scores, axis=-1)
        ctx = jnp.einsum("bhqk,bhkd->bhqd", p, v)
        return jnp.einsum("bhqd,hdm->bqm", ctx, w_o)

    def _B_ref(x, w1, b1, w2, b2):
        h = jnp.einsum("bsd,df->bsf", x, w1) + b1
        h = _gelu(h)
        return jnp.einsum("bsf,fd->bsd", h, w2) + b2

    x = A_x
    xn = _layernorm(x, axis=-1)
    s = _A_ref(xn, A_c_kv, A_w_q, A_w_uk, A_w_uv, A_w_o)
    g = _silu(_B_ref(xn, B_w1, B_b1, B_w2, B_b2))
    return x + s * g
```

```python
import functools

import jax
import jax.numpy as jnp
from jax import lax
import jax.experimental.pallas as pl
import jax.experimental.pallas.tpu as pltpu

F32 = jnp.float32
BF16 = jnp.bfloat16

HG = 16
LANES = 128
TK = 2048
KV_DMA_ROWS = 4096
NT = (((1,), (1,)), ((), ()))


def _kernel(x_hbm, ckv_hbm, wq_hbm, wuk_hbm, wuv_hbm, wo_hbm,
            w1_hbm, b1_hbm, w2_hbm, b2_hbm,
            o_ref,
            x_v, ckv_v, wq_v, wuk_v, wuv_v, wo_v, w1_v, b1_v, w2_v, b2_v,
            e_v, et_v, lhs_v, qa_v, m_v, l_v, acc_v,
            sem, kv_sem,
            *, B, S, C, H, D, M, FF, wo_splits):
    n_kv = S // KV_DMA_ROWS
    NHG = H // HG
    G = C // LANES
    R = B * HG
    W = LANES * HG

    cp_x = pltpu.make_async_copy(x_hbm, x_v, sem.at[0])
    cp_wq = pltpu.make_async_copy(wq_hbm, wq_v, sem.at[1])
    cp_wuk = pltpu.make_async_copy(wuk_hbm, wuk_v, sem.at[2])
    cp_b1 = pltpu.make_async_copy(b1_hbm, b1_v, sem.at[3])
    cp_b2 = pltpu.make_async_copy(b2_hbm, b2_v, sem.at[4])
    cp_w1 = pltpu.make_async_copy(w1_hbm, w1_v, sem.at[5])
    cp_w2 = pltpu.make_async_copy(w2_hbm, w2_v, sem.at[6])
    cp_wuv = pltpu.make_async_copy(wuv_hbm, wuv_v, sem.at[7])
    cp_wo = [
        pltpu.make_async_copy(wo_hbm.at[pl.ds(h0, h1 - h0)],
                              wo_v.at[pl.ds(h0, h1 - h0)], sem.at[8 + k])
        for k, (h0, h1) in enumerate(wo_splits)
    ]

    def kv_copy(b, j):
        rows = pl.ds(j * KV_DMA_ROWS, KV_DMA_ROWS)
        return pltpu.make_async_copy(ckv_hbm.at[b, rows], ckv_v.at[b, rows],
                                     kv_sem.at[b * n_kv + j])

    cp_x.start()
    cp_wq.start()
    cp_wuk.start()
    for b in range(B):
        for j in range(n_kv):
            kv_copy(b, j).start()
    cp_b1.start()
    cp_b2.start()
    cp_w1.start()
    cp_w2.start()
    cp_wuv.start()
    for cp in cp_wo:
        cp.start()

    e_v[...] = (lax.broadcasted_iota(jnp.int32, (LANES, W), 0)
                == lax.broadcasted_iota(jnp.int32, (LANES, W), 1) // HG
                ).astype(F32).astype(BF16)
    et_v[...] = (lax.broadcasted_iota(jnp.int32, (W, LANES), 0) // HG
                 == lax.broadcasted_iota(jnp.int32, (W, LANES), 1)
                 ).astype(F32).astype(BF16)

    def diag_mask(rows):
        return (lax.broadcasted_iota(jnp.int32, (rows, W), 0) % HG
                == lax.broadcasted_iota(jnp.int32, (rows, W), 1) % HG)

    def expand(a):
        st = jnp.concatenate([a[:, g * LANES:(g + 1) * LANES] for g in range(G)], axis=0)
        rep = jnp.dot(st, e_v[...], preferred_element_type=F32)
        return jnp.where(diag_mask(G * R), rep, 0.0).astype(BF16)

    def head_group(w_ref, g, hg):
        return w_ref[g * LANES:(g + 1) * LANES, hg * HG:(hg + 1) * HG, :].reshape(W, D)

    cp_x.wait()
    xs = [x_v[b].astype(F32) for b in range(B)]
    xns = []
    for xb in xs:
        mu = jnp.mean(xb, axis=-1, keepdims=True)
        xc = xb - mu
        var = jnp.mean(xc * xc, axis=-1, keepdims=True)
        xns.append(xc / jnp.sqrt(var + 1e-5))
    xrows = jnp.concatenate(
        [jnp.broadcast_to(xn, (HG, M)) for xn in xns], axis=0).astype(BF16)

    lq = expand(xrows)
    cp_wq.wait()
    scale = D ** -0.5
    qs = []
    for hg in range(NHG):
        acc = jnp.zeros((R, D), F32)
        for g in range(G):
            acc += jnp.dot(lq[g * R:(g + 1) * R], head_group(wq_v, g, hg),
                           preferred_element_type=F32)
        qs.append((acc * scale).astype(BF16))

    cp_wuk.wait()
    dm = diag_mask(R)
    for hg in range(NHG):
        for g in range(G):
            st = lax.dot_general(qs[hg], head_group(wuk_v, g, hg), NT,
                                 preferred_element_type=F32)
            k = hg * G + g
            lhs_v[k * R:(k + 1) * R, :] = jnp.where(dm, st, 0.0).astype(BF16)
    qa = jnp.dot(lhs_v[...], et_v[...], preferred_element_type=F32).astype(BF16)
    for b in range(B):
        for hg in range(NHG):
            for g in range(G):
                r0 = (hg * G + g) * R + b * HG
                qa_v[b, hg * HG:(hg + 1) * HG, g * LANES:(g + 1) * LANES] = qa[r0:r0 + HG]

    m_v[...] = jnp.full(m_v.shape, -jnp.inf, F32)
    l_v[...] = jnp.zeros(l_v.shape, F32)
    acc_v[...] = jnp.zeros(acc_v.shape, F32)
    sub = KV_DMA_ROWS // TK

    def kv_step(t, carry):
        b = t // (S // TK)
        j = t % (S // TK)

        @pl.when(j % sub == 0)
        def _():
            kv_copy(b, j // sub).wait()

        c = ckv_v[b, pl.ds(pl.multiple_of(j * TK, TK), TK), :]
        s = lax.dot_general(qa_v[b], c, NT, preferred_element_type=F32)
        m_old = m_v[b]
        m_new = jnp.maximum(m_old, jnp.max(s, axis=-1, keepdims=True))
        alpha = jnp.exp(m_old - m_new)
        p = jnp.exp(s - m_new)
        l_v[b] = alpha * l_v[b] + jnp.sum(p, axis=-1, keepdims=True)
        acc_v[b] = alpha * acc_v[b] + jnp.dot(p.astype(BF16), c, preferred_element_type=F32)
        m_v[b] = m_new
        return carry

    lax.fori_loop(0, B * (S // TK), kv_step, 0)

    ctxc = [(acc_v[b] / l_v[b]).astype(BF16) for b in range(B)]
    for hg in range(NHG):
        a = jnp.concatenate([ctxc[b][hg * HG:(hg + 1) * HG] for b in range(B)], axis=0)
        lhs_v[hg * G * R:(hg + 1) * G * R, :] = expand(a)

    cp_b1.wait()
    cp_b2.wait()
    cp_w1.wait()
    hid = jnp.dot(xrows, w1_v[...], preferred_element_type=F32)
    hid = hid + b1_v[...].astype(F32).reshape(1, FF)
    hid = jax.nn.gelu(hid, approximate=True).astype(BF16)
    cp_w2.wait()
    y = jnp.dot(hid, w2_v[...], preferred_element_type=F32)
    y = y + b2_v[...].astype(F32).reshape(1, M)
    gate = y * jax.nn.sigmoid(y)

    cp_wuv.wait()
    ctx = []
    for hg in range(NHG):
        acc = jnp.zeros((R, D), F32)
        for g in range(G):
            k = hg * G + g
            acc += jnp.dot(lhs_v[k * R:(k + 1) * R, :], head_group(wuv_v, g, hg),
                           preferred_element_type=F32)
        ctx.append(acc)

    row_i = lax.broadcasted_iota(jnp.int32, (R, D), 0) % HG
    sacc = jnp.zeros((R, M), F32)
    for cp, (h0, h1) in zip(cp_wo, wo_splits):
        lo = jnp.concatenate(
            [jnp.where(row_i == h % HG, ctx[h // HG], 0.0).astype(BF16)
             for h in range(h0, h1)], axis=1)
        cp.wait()
        sacc += jnp.dot(lo, wo_v[h0:h1].reshape((h1 - h0) * D, M),
                        preferred_element_type=F32)
    for b in range(B):
        s_b = jnp.sum(sacc[b * HG:(b + 1) * HG], axis=0, keepdims=True)
        o_ref[b] = (xs[b] + s_b * gate[b * HG:b * HG + 1]).astype(o_ref.dtype)


@jax.jit
def pallas_recurrent_scan__compressed_kv_cla__dense_activation_gelu__decode_kernel(
    A_x: jax.Array,
    A_c_kv: jax.Array,
    A_w_q: jax.Array,
    A_w_uk: jax.Array,
    A_w_uv: jax.Array,
    A_w_o: jax.Array,
    B_x: jax.Array,
    B_w1: jax.Array,
    B_b1: jax.Array,
    B_w2: jax.Array,
    B_b2: jax.Array,
):
    del B_x
    B, Sq, M = A_x.shape
    _, S, C = A_c_kv.shape
    _, H, D = A_w_q.shape
    FF = B_w1.shape[1]
    assert Sq == 1 and M == C and D == LANES and H % HG == 0
    wo_splits = ((0, 24), (24, 30), (30, 32))
    G = C // LANES
    R = B * HG
    W = LANES * HG

    kernel = functools.partial(_kernel, B=B, S=S, C=C, H=H, D=D, M=M, FF=FF,
                               wo_splits=wo_splits)
    hbm = pl.BlockSpec(memory_space=pl.ANY)
    return pl.pallas_call(
        kernel,
        out_shape=jax.ShapeDtypeStruct(A_x.shape, A_x.dtype),
        in_specs=[hbm] * 10,
        out_specs=pl.BlockSpec(memory_space=pltpu.VMEM),
        scratch_shapes=[
            pltpu.VMEM(A_x.shape, BF16),
            pltpu.VMEM(A_c_kv.shape, BF16),
            pltpu.VMEM(A_w_q.shape, BF16),
            pltpu.VMEM(A_w_uk.shape, BF16),
            pltpu.VMEM(A_w_uv.shape, BF16),
            pltpu.VMEM(A_w_o.shape, BF16),
            pltpu.VMEM(B_w1.shape, BF16),
            pltpu.VMEM(B_b1.shape, BF16),
            pltpu.VMEM(B_w2.shape, BF16),
            pltpu.VMEM(B_b2.shape, BF16),
            pltpu.VMEM((LANES, W), BF16),
            pltpu.VMEM((W, LANES), BF16),
            pltpu.VMEM(((H // HG) * G * R, W), BF16),
            pltpu.VMEM((B, H, C), BF16),
            pltpu.VMEM((B, H, 1), F32),
            pltpu.VMEM((B, H, 1), F32),
            pltpu.VMEM((B, H, C), F32),
            pltpu.SemaphoreType.DMA((8 + len(wo_splits),)),
            pltpu.SemaphoreType.DMA((B * (S // KV_DMA_ROWS),)),
        ],
        compiler_params=pltpu.CompilerParams(vmem_limit_bytes=100 * 1024 * 1024),
    )(A_x, A_c_kv, A_w_q, A_w_uk, A_w_uv, A_w_o, B_w1, B_b1, B_w2, B_b2)
```

```python
import functools

import jax
import jax.numpy as jnp
from jax import lax
import jax.experimental.pallas as pl
import jax.experimental.pallas.tpu as pltpu

F32 = jnp.float32
BF16 = jnp.bfloat16

HG = 16
LANES = 128
TK = 2048
KV_DMA_ROWS = 4096
NT = (((1,), (1,)), ((), ()))


def _kernel(x_hbm, ckv_hbm, wq_hbm, wuk_hbm, wuv_hbm, wo_hbm,
            w1_hbm, b1_hbm, w2_hbm, b2_hbm,
            o_ref,
            x_v, ckv_v, wq_v, wuk_v, wuv_v, wo_v, w1_v, b1_v, w2_v, b2_v,
            e_v, et_v, lhs_v, qa_v, m_v, l_v, acc_v, s_v,
            sem,
            *, B, S, C, H, D, M, FF, wo_splits):
    n_kv = S // KV_DMA_ROWS
    NHG = H // HG
    G = C // LANES
    R = B * HG
    W = LANES * HG

    cp_x = pltpu.make_async_copy(x_hbm, x_v, sem.at[0])
    cp_wq = pltpu.make_async_copy(wq_hbm, wq_v, sem.at[1])
    cp_wuk = pltpu.make_async_copy(wuk_hbm, wuk_v, sem.at[2])
    cp_b1 = pltpu.make_async_copy(b1_hbm, b1_v, sem.at[3])
    cp_b2 = pltpu.make_async_copy(b2_hbm, b2_v, sem.at[4])
    cp_w1 = pltpu.make_async_copy(w1_hbm, w1_v, sem.at[5])
    cp_w2 = pltpu.make_async_copy(w2_hbm, w2_v, sem.at[6])
    cp_wuv = pltpu.make_async_copy(wuv_hbm, wuv_v, sem.at[7])
    cp_wo = [
        pltpu.make_async_copy(wo_hbm.at[pl.ds(h0, h1 - h0)],
                              wo_v.at[pl.ds(h0, h1 - h0)], sem.at[8 + k])
        for k, (h0, h1) in enumerate(wo_splits)
    ]

    def kv_copy(b, j):
        rows = pl.ds(j * KV_DMA_ROWS, KV_DMA_ROWS)
        return pltpu.make_async_copy(ckv_hbm.at[b, rows], ckv_v.at[b, rows],
                                     sem.at[8 + len(wo_splits) + b * n_kv + j])

    cp_x.start()
    cp_wq.start()
    cp_wuk.start()
    for b in range(B):
        for j in range(n_kv):
            kv_copy(b, j).start()
    cp_b1.start()
    cp_b2.start()
    cp_w1.start()
    cp_w2.start()
    cp_wuv.start()
    for cp in cp_wo:
        cp.start()

    e_v[...] = (lax.broadcasted_iota(jnp.int32, (LANES, W), 0)
                == lax.broadcasted_iota(jnp.int32, (LANES, W), 1) // HG
                ).astype(F32).astype(BF16)
    et_v[...] = (lax.broadcasted_iota(jnp.int32, (W, LANES), 0) // HG
                 == lax.broadcasted_iota(jnp.int32, (W, LANES), 1)
                 ).astype(F32).astype(BF16)

    def diag_mask(rows):
        return (lax.broadcasted_iota(jnp.int32, (rows, W), 0) % HG
                == lax.broadcasted_iota(jnp.int32, (rows, W), 1) % HG)

    def expand(a):
        st = jnp.concatenate([a[:, g * LANES:(g + 1) * LANES] for g in range(G)], axis=0)
        rep = jnp.dot(st, e_v[...], preferred_element_type=F32)
        return jnp.where(diag_mask(G * R), rep, 0.0).astype(BF16)

    def head_group(w_ref, g, hg):
        return w_ref[g * LANES:(g + 1) * LANES, hg * HG:(hg + 1) * HG, :].reshape(W, D)

    cp_x.wait()
    x32 = x_v[...].astype(F32)
    xs = [x32[b:b + 1] for b in range(B)]
    xns = []
    for xb in xs:
        mu = jnp.mean(xb, axis=-1, keepdims=True)
        xc = xb - mu
        var = jnp.mean(xc * xc, axis=-1, keepdims=True)
        xns.append(xc / jnp.sqrt(var + 1e-5))
    xrows = jnp.concatenate(
        [jnp.broadcast_to(xn, (HG, M)) for xn in xns], axis=0).astype(BF16)

    lq = expand(xrows)
    cp_wq.wait()
    scale = D ** -0.5
    qs = []
    for hg in range(NHG):
        acc = jnp.zeros((R, D), F32)
        for g in range(G):
            acc += jnp.dot(lq[g * R:(g + 1) * R], head_group(wq_v, g, hg),
                           preferred_element_type=F32)
        qs.append((acc * scale).astype(BF16))

    cp_wuk.wait()
    dm = diag_mask(R)
    for hg in range(NHG):
        for g in range(G):
            st = lax.dot_general(qs[hg], head_group(wuk_v, g, hg), NT,
                                 preferred_element_type=F32)
            k = hg * G + g
            lhs_v[k * R:(k + 1) * R, :] = jnp.where(dm, st, 0.0).astype(BF16)
    qa = jnp.dot(lhs_v[...], et_v[...], preferred_element_type=F32).astype(BF16)
    for b in range(B):
        for hg in range(NHG):
            for g in range(G):
                r0 = (hg * G + g) * R + b * HG
                qa_v[b, hg * HG:(hg + 1) * HG, g * LANES:(g + 1) * LANES] = qa[r0:r0 + HG]

    m_v[...] = jnp.full(m_v.shape, -jnp.inf, F32)
    l_v[...] = jnp.zeros(l_v.shape, F32)
    acc_v[...] = jnp.zeros(acc_v.shape, F32)
    sub = KV_DMA_ROWS // TK

    def kv_step(t, carry):
        b = t // (S // TK)
        j = t % (S // TK)

        @pl.when(j % sub == 0)
        def _():
            kv_copy(b, j // sub).wait()

        c = ckv_v[b, pl.ds(pl.multiple_of(j * TK, TK), TK), :]
        s = lax.dot_general(qa_v[b], c, NT, preferred_element_type=F32)
        m_old = m_v[b]
        m_new = jnp.maximum(m_old, jnp.max(s, axis=-1, keepdims=True))
        alpha = jnp.exp(m_old - m_new)
        p = jnp.exp(s - m_new)
        l_v[b] = alpha * l_v[b] + jnp.sum(p, axis=-1, keepdims=True)
        acc_v[b] = alpha * acc_v[b] + jnp.dot(p.astype(BF16), c, preferred_element_type=F32)
        m_v[b] = m_new
        return carry

    lax.fori_loop(0, B * (S // TK), kv_step, 0)

    ctxc = [(acc_v[b] / l_v[b]).astype(BF16) for b in range(B)]
    for hg in range(NHG):
        a = jnp.concatenate([ctxc[b][hg * HG:(hg + 1) * HG] for b in range(B)], axis=0)
        lhs_v[hg * G * R:(hg + 1) * G * R, :] = expand(a)

    cp_b1.wait()
    cp_b2.wait()
    cp_w1.wait()
    hid = jnp.dot(xrows, w1_v[...], preferred_element_type=F32)
    hid = hid + b1_v[...].astype(F32).reshape(1, FF)
    hid = jax.nn.gelu(hid, approximate=True).astype(BF16)
    cp_w2.wait()
    y = jnp.dot(hid, w2_v[...], preferred_element_type=F32)
    y = y + b2_v[...].astype(F32).reshape(1, M)
    gate = y * jax.nn.sigmoid(y)

    cp_wuv.wait()
    ctx = []
    for hg in range(NHG):
        acc = jnp.zeros((R, D), F32)
        for g in range(G):
            k = hg * G + g
            acc += jnp.dot(lhs_v[k * R:(k + 1) * R, :], head_group(wuv_v, g, hg),
                           preferred_element_type=F32)
        ctx.append(acc)

    row_i = lax.broadcasted_iota(jnp.int32, (R, D), 0) % HG
    for k, (cp, (h0, h1)) in enumerate(zip(cp_wo, wo_splits)):
        lo = jnp.concatenate(
            [jnp.where(row_i == h % HG, ctx[h // HG], 0.0).astype(BF16)
             for h in range(h0, h1)], axis=1)
        cp.wait()
        part = jnp.dot(lo, wo_v[h0:h1].reshape((h1 - h0) * D, M),
                       preferred_element_type=F32)
        if k > 0:
            part = part + s_v[...]
        if k + 1 < len(wo_splits):
            s_v[...] = part
    outs = []
    for b in range(B):
        s_b = jnp.sum(part[b * HG:(b + 1) * HG], axis=0, keepdims=True)
        outs.append(xs[b] + s_b * gate[b * HG:b * HG + 1])
    o_ref[...] = jnp.concatenate(outs, axis=0).astype(o_ref.dtype)


@jax.jit
def pallas_recurrent_scan__compressed_kv_cla__dense_activation_gelu__decode_kernel(
    A_x: jax.Array,
    A_c_kv: jax.Array,
    A_w_q: jax.Array,
    A_w_uk: jax.Array,
    A_w_uv: jax.Array,
    A_w_o: jax.Array,
    B_x: jax.Array,
    B_w1: jax.Array,
    B_b1: jax.Array,
    B_w2: jax.Array,
    B_b2: jax.Array,
):
    del B_x
    B, Sq, M = A_x.shape
    _, S, C = A_c_kv.shape
    _, H, D = A_w_q.shape
    FF = B_w1.shape[1]
    assert Sq == 1 and M == C and D == LANES and H % HG == 0
    wo_splits = ((0, 24), (24, 30), (30, 32))
    G = C // LANES
    R = B * HG
    W = LANES * HG

    kernel = functools.partial(_kernel, B=B, S=S, C=C, H=H, D=D, M=M, FF=FF,
                               wo_splits=wo_splits)
    hbm = pl.BlockSpec(memory_space=pl.ANY)
    return pl.pallas_call(
        kernel,
        out_shape=jax.ShapeDtypeStruct((B, M), A_x.dtype),
        in_specs=[hbm] * 10,
        out_specs=pl.BlockSpec(memory_space=pltpu.VMEM),
        scratch_shapes=[
            pltpu.VMEM((B, M), BF16),
            pltpu.VMEM(A_c_kv.shape, BF16),
            pltpu.VMEM(A_w_q.shape, BF16),
            pltpu.VMEM(A_w_uk.shape, BF16),
            pltpu.VMEM(A_w_uv.shape, BF16),
            pltpu.VMEM(A_w_o.shape, BF16),
            pltpu.VMEM(B_w1.shape, BF16),
            pltpu.VMEM(B_b1.shape, BF16),
            pltpu.VMEM(B_w2.shape, BF16),
            pltpu.VMEM(B_b2.shape, BF16),
            pltpu.VMEM((LANES, W), BF16),
            pltpu.VMEM((W, LANES), BF16),
            pltpu.VMEM(((H // HG) * G * R, W), BF16),
            pltpu.VMEM((B, H, C), BF16),
            pltpu.VMEM((B, H, 1), F32),
            pltpu.VMEM((B, H, 1), F32),
            pltpu.VMEM((B, H, C), F32),
            pltpu.VMEM((R, M), F32),
            pltpu.SemaphoreType.DMA((8 + len(wo_splits) + B * (S // KV_DMA_ROWS),)),
        ],
        compiler_params=pltpu.CompilerParams(vmem_limit_bytes=100 * 1024 * 1024,
                                             disable_semaphore_checks=True),
    )(A_x.reshape(B, M), A_c_kv, A_w_q, A_w_uk, A_w_uv, A_w_o,
      B_w1, B_b1, B_w2, B_b2).reshape(B, Sq, M)
```

```python
import functools

import jax
import jax.numpy as jnp
from jax import lax
import jax.experimental.pallas as pl
import jax.experimental.pallas.tpu as pltpu

F32 = jnp.float32
BF16 = jnp.bfloat16

LANES = 128
SUB = 8
HG = 16
TK = 2048
KV_DMA_ROWS = 4096
STAGE_ROWS = 144
STAGE_PIECES = 11
STAGE_SLOTS = 4
WO_MXU_TAIL = (512,)
WO_VPU_TAIL = (128, 96, 32)
NT = (((1,), (1,)), ((), ()))


def _kernel(x_hbm, ckv_hbm, wq_hbm, wuk_hbm, wuv_hbm, wo_hbm,
            w1_hbm, b1_hbm, w2_hbm, b2_hbm,
            o_ref,
            x_v, ckv_v, wq_v, wuk_v, wuv_v, wo_v, w1_v, b1_v, w2_v, b2_v,
            e_v, et_v, lhs_v, qa_v, m_v, l_v, acc_v, s_v, cb_v, stage,
            sem,
            *, B, S, C, H, D, M, FF, wo_splits):
    n_kv = S // KV_DMA_ROWS
    NHG = H // HG
    G = C // LANES
    R = B * HG
    W = LANES * HG
    n_vpu = len(WO_VPU_TAIL)
    vpu_heads = sum(WO_VPU_TAIL) // D
    KV0 = 8 + len(wo_splits)
    ST0 = KV0 + B * n_kv

    cp_x = pltpu.make_async_copy(x_hbm, x_v, sem.at[0])
    cp_wq = pltpu.make_async_copy(wq_hbm, wq_v, sem.at[1])
    cp_wuk = pltpu.make_async_copy(wuk_hbm, wuk_v, sem.at[2])
    cp_b1 = pltpu.make_async_copy(b1_hbm, b1_v, sem.at[3])
    cp_b2 = pltpu.make_async_copy(b2_hbm, b2_v, sem.at[4])
    cp_w1 = pltpu.make_async_copy(w1_hbm, w1_v, sem.at[5])
    cp_w2 = pltpu.make_async_copy(w2_hbm, w2_v, sem.at[6])
    cp_wuv = pltpu.make_async_copy(wuv_hbm, wuv_v, sem.at[7])
    cp_wo = [
        pltpu.make_async_copy(wo_hbm.at[pl.ds(r0, r1 - r0)],
                              wo_v.at[pl.ds(r0, r1 - r0)], sem.at[8 + k])
        for k, (r0, r1) in enumerate(wo_splits)
    ]

    def kv_copy(b, j):
        rows = pl.ds(j * KV_DMA_ROWS, KV_DMA_ROWS)
        return pltpu.make_async_copy(ckv_hbm.at[b, rows], ckv_v.at[b, rows],
                                     sem.at[KV0 + b * n_kv + j])

    def stage_slot(p):
        return stage.at[pl.ds((p % STAGE_SLOTS) * STAGE_ROWS, STAGE_ROWS)]

    def stage_in(p):
        return pltpu.make_async_copy(wo_hbm.at[pl.ds(p * STAGE_ROWS, STAGE_ROWS)],
                                     stage_slot(p), sem.at[ST0 + 2 * p])

    def stage_out(p):
        return pltpu.make_async_copy(stage_slot(p),
                                     wo_v.at[pl.ds(p * STAGE_ROWS, STAGE_ROWS)],
                                     sem.at[ST0 + 2 * p + 1])

    def stage_step(j):
        if j - 1 < STAGE_PIECES:
            stage_in(j - 1).wait()
            stage_out(j - 1).start()
        if j + 1 < STAGE_PIECES:
            if j + 1 >= STAGE_SLOTS:
                stage_out(j + 1 - STAGE_SLOTS).wait()
            stage_in(j + 1).start()

    cp_x.start()
    cp_wq.start()
    stage_in(0).start()
    stage_in(1).start()
    cp_wuk.start()
    for b in range(B):
        for j in range(n_kv):
            kv_copy(b, j).start()
    cp_b1.start()
    cp_b2.start()
    cp_w1.start()
    cp_w2.start()
    cp_wuv.start()
    for cp in cp_wo:
        cp.start()

    e_v[...] = (lax.broadcasted_iota(jnp.int32, (LANES, W), 0)
                == lax.broadcasted_iota(jnp.int32, (LANES, W), 1) // HG
                ).astype(F32).astype(BF16)
    et_v[...] = (lax.broadcasted_iota(jnp.int32, (W, LANES), 0) // HG
                 == lax.broadcasted_iota(jnp.int32, (W, LANES), 1)
                 ).astype(F32).astype(BF16)

    def diag_mask(rows):
        return (lax.broadcasted_iota(jnp.int32, (rows, W), 0) % HG
                == lax.broadcasted_iota(jnp.int32, (rows, W), 1) % HG)

    def expand(a):
        st = jnp.concatenate([a[:, g * LANES:(g + 1) * LANES] for g in range(G)], axis=0)
        rep = jnp.dot(st, e_v[...], preferred_element_type=F32)
        return jnp.where(diag_mask(G * R), rep, 0.0).astype(BF16)

    def head_group(w_ref, g, hg):
        return w_ref[g * LANES:(g + 1) * LANES, hg * HG:(hg + 1) * HG, :].reshape(W, D)

    cp_x.wait()
    x32 = x_v[...].astype(F32)
    xs = [x32[b:b + 1] for b in range(B)]
    xns = []
    for xb in xs:
        mu = jnp.mean(xb, axis=-1, keepdims=True)
        xc = xb - mu
        var = jnp.mean(xc * xc, axis=-1, keepdims=True)
        xns.append(xc / jnp.sqrt(var + 1e-5))
    xrows = jnp.concatenate(
        [jnp.broadcast_to(xn, (HG, M)) for xn in xns], axis=0).astype(BF16)

    lq = expand(xrows)
    cp_wq.wait()
    stage_step(1)
    scale = D ** -0.5
    qs = []
    for hg in range(NHG):
        acc = jnp.zeros((R, D), F32)
        for g in range(G):
            acc += jnp.dot(lq[g * R:(g + 1) * R], head_group(wq_v, g, hg),
                           preferred_element_type=F32)
        qs.append((acc * scale).astype(BF16))

    cp_wuk.wait()
    stage_step(2)
    dm = diag_mask(R)
    for hg in range(NHG):
        for g in range(G):
            st = lax.dot_general(qs[hg], head_group(wuk_v, g, hg), NT,
                                 preferred_element_type=F32)
            k = hg * G + g
            lhs_v[k * R:(k + 1) * R, :] = jnp.where(dm, st, 0.0).astype(BF16)
    qa = jnp.dot(lhs_v[...], et_v[...], preferred_element_type=F32).astype(BF16)
    for b in range(B):
        for hg in range(NHG):
            for g in range(G):
                r0 = (hg * G + g) * R + b * HG
                qa_v[b, hg * HG:(hg + 1) * HG, g * LANES:(g + 1) * LANES] = qa[r0:r0 + HG]

    m_v[...] = jnp.full(m_v.shape, -jnp.inf, F32)
    l_v[...] = jnp.zeros(l_v.shape, F32)
    acc_v[...] = jnp.zeros(acc_v.shape, F32)
    sub = KV_DMA_ROWS // TK

    def kv_step(t, carry):
        b = t // (S // TK)
        j = t % (S // TK)

        @pl.when(j % sub == 0)
        def _():
            kv_copy(b, j // sub).wait()

        for k in range(B * n_kv):
            pl.when(t == k * sub)(functools.partial(stage_step, 3 + k))

        c = ckv_v[b, pl.ds(pl.multiple_of(j * TK, TK), TK), :]
        s = lax.dot_general(qa_v[b], c, NT, preferred_element_type=F32)
        m_old = m_v[b]
        m_new = jnp.maximum(m_old, jnp.max(s, axis=-1, keepdims=True))
        alpha = jnp.exp(m_old - m_new)
        p = jnp.exp(s - m_new)
        l_v[b] = alpha * l_v[b] + jnp.sum(p, axis=-1, keepdims=True)
        acc_v[b] = alpha * acc_v[b] + jnp.dot(p.astype(BF16), c, preferred_element_type=F32)
        m_v[b] = m_new
        return carry

    lax.fori_loop(0, B * (S // TK), kv_step, 0)

    ctxc = [(acc_v[b] / l_v[b]).astype(BF16) for b in range(B)]
    for hg in range(NHG):
        a = jnp.concatenate([ctxc[b][hg * HG:(hg + 1) * HG] for b in range(B)], axis=0)
        lhs_v[hg * G * R:(hg + 1) * G * R, :] = expand(a)

    cp_b1.wait()
    cp_b2.wait()
    cp_w1.wait()
    hid = jnp.dot(xrows, w1_v[...], preferred_element_type=F32)
    hid = hid + b1_v[...].astype(F32).reshape(1, FF)
    hid = jax.nn.gelu(hid, approximate=True).astype(BF16)
    cp_w2.wait()
    y = jnp.dot(hid, w2_v[...], preferred_element_type=F32)
    y = y + b2_v[...].astype(F32).reshape(1, M)
    s_v[...] = y * jax.nn.sigmoid(y)
    for j in range(3 + B * n_kv, STAGE_PIECES + 1):
        stage_step(j)
    gate = s_v[...]

    cp_wuv.wait()
    ctx = []
    for hg in range(NHG):
        acc = jnp.zeros((R, D), F32)
        for g in range(G):
            k = hg * G + g
            acc += jnp.dot(lhs_v[k * R:(k + 1) * R, :], head_group(wuv_v, g, hg),
                           preferred_element_type=F32)
        ctx.append(acc)

    row_i = lax.broadcasted_iota(jnp.int32, (R, D), 0) % HG
    lo = jnp.concatenate(
        [jnp.where(row_i == h % HG, ctx[h // HG], 0.0).astype(BF16)
         for h in range(H - vpu_heads)], axis=1)
    for b in range(B):
        for u in range(vpu_heads):
            i = b * HG + HG - vpu_heads + u
            row = ctx[NHG - 1][i:i + 1, :].astype(BF16).astype(F32)
            cb_v[b, u * D:(u + 1) * D] = jnp.transpose(jnp.broadcast_to(row, (LANES, D)))

    for p in range(max(STAGE_PIECES - STAGE_SLOTS, 0), STAGE_PIECES):
        stage_out(p).wait()
    r_staged = STAGE_PIECES * STAGE_ROWS
    s_v[...] = jnp.dot(lo[:, :r_staged], wo_v[:r_staged], preferred_element_type=F32)
    n_mxu = len(wo_splits) - n_vpu
    for k in range(n_mxu):
        r0, r1 = wo_splits[k]
        cp_wo[k].wait()
        part = s_v[...] + jnp.dot(lo[:, r0:r1], wo_v[r0:r1], preferred_element_type=F32)
        if k + 1 < n_mxu:
            s_v[...] = part
    for b in range(B):
        s_v[b * SUB:(b + 1) * SUB, :] = (part[b * HG:b * HG + SUB]
                                         + part[b * HG + SUB:(b + 1) * HG])
    v0 = (H - vpu_heads) * D
    for k in range(n_mxu, len(wo_splits)):
        r0, r1 = wo_splits[k]
        cp_wo[k].wait()
        w32 = wo_v[r0:r1].astype(F32)
        accs = []
        for b in range(B):
            cb = cb_v[b, r0 - v0:r1 - v0, :]
            prod = w32 * jnp.concatenate([cb] * (M // LANES), axis=1)
            a = s_v[b * SUB:(b + 1) * SUB, :]
            for u in range((r1 - r0) // SUB):
                a = a + prod[u * SUB:(u + 1) * SUB]
            accs.append(a)
            if k + 1 < len(wo_splits):
                s_v[b * SUB:(b + 1) * SUB, :] = a
    outs = [xs[b] + jnp.sum(accs[b], axis=0, keepdims=True) * gate[b * HG:b * HG + 1]
            for b in range(B)]
    o_ref[...] = jnp.concatenate(outs, axis=0).astype(o_ref.dtype)


@jax.jit
def pallas_recurrent_scan__compressed_kv_cla__dense_activation_gelu__decode_kernel(
    A_x: jax.Array,
    A_c_kv: jax.Array,
    A_w_q: jax.Array,
    A_w_uk: jax.Array,
    A_w_uv: jax.Array,
    A_w_o: jax.Array,
    B_x: jax.Array,
    B_w1: jax.Array,
    B_b1: jax.Array,
    B_w2: jax.Array,
    B_b2: jax.Array,
):
    del B_x
    B, Sq, M = A_x.shape
    _, S, C = A_c_kv.shape
    _, H, D = A_w_q.shape
    FF = B_w1.shape[1]
    assert Sq == 1 and M == C and D == LANES and H % HG == 0 and S % KV_DMA_ROWS == 0
    assert sum(WO_VPU_TAIL) % D == 0 and sum(WO_VPU_TAIL) <= HG * D
    G = C // LANES
    R = B * HG
    W = LANES * HG

    r = STAGE_PIECES * STAGE_ROWS
    sizes = (H * D - r - sum(WO_MXU_TAIL) - sum(WO_VPU_TAIL),) + WO_MXU_TAIL + WO_VPU_TAIL
    wo_splits = []
    for n in sizes:
        wo_splits.append((r, r + n))
        r += n
    n_sem = 8 + len(wo_splits) + B * (S // KV_DMA_ROWS) + 2 * STAGE_PIECES

    kernel = functools.partial(_kernel, B=B, S=S, C=C, H=H, D=D, M=M, FF=FF,
                               wo_splits=tuple(wo_splits))
    hbm = pl.BlockSpec(memory_space=pl.ANY)
    out = pl.pallas_call(
        kernel,
        out_shape=jax.ShapeDtypeStruct((B, M), A_x.dtype),
        in_specs=[hbm] * 10,
        out_specs=pl.BlockSpec(memory_space=pltpu.VMEM),
        scratch_shapes=[
            pltpu.VMEM((B, M), BF16),
            pltpu.VMEM(A_c_kv.shape, BF16),
            pltpu.VMEM(A_w_q.shape, BF16),
            pltpu.VMEM(A_w_uk.shape, BF16),
            pltpu.VMEM(A_w_uv.shape, BF16),
            pltpu.VMEM((H * D, M), BF16),
            pltpu.VMEM(B_w1.shape, BF16),
            pltpu.VMEM(B_b1.shape, BF16),
            pltpu.VMEM(B_w2.shape, BF16),
            pltpu.VMEM(B_b2.shape, BF16),
            pltpu.VMEM((LANES, W), BF16),
            pltpu.VMEM((W, LANES), BF16),
            pltpu.VMEM(((H // HG) * G * R, W), BF16),
            pltpu.VMEM((B, H, C), BF16),
            pltpu.VMEM((B, H, 1), F32),
            pltpu.VMEM((B, H, 1), F32),
            pltpu.VMEM((B, H, C), F32),
            pltpu.VMEM((R, M), F32),
            pltpu.VMEM((B, sum(WO_VPU_TAIL), LANES), F32),
            pltpu.SMEM((STAGE_SLOTS * STAGE_ROWS, M), BF16),
            pltpu.SemaphoreType.DMA((n_sem,)),
        ],
        compiler_params=pltpu.CompilerParams(vmem_limit_bytes=100 * 1024 * 1024,
                                             disable_semaphore_checks=True),
    )(A_x.reshape(B, M), A_c_kv, A_w_q, A_w_uk, A_w_uv, A_w_o.reshape(H * D, M),
      B_w1, B_b1, B_w2, B_b2)
    return out.reshape(B, Sq, M)
```

```python
import functools

import jax
import jax.numpy as jnp
from jax import lax
import jax.experimental.pallas as pl
import jax.experimental.pallas.tpu as pltpu

F32 = jnp.float32
BF16 = jnp.bfloat16

LANES = 128
SUB = 8
HG = 16
TK = 2048
KV_DMA_ROWS = 4096
STAGE_ROWS = 144
STAGE_PIECES = 11
STAGE_SLOTS = 4
WO_MXU_TAIL = (512,)
WO_VPU_TAIL = (128, 96, 32)
NT = (((1,), (1,)), ((), ()))


def _kernel(x_hbm, ckv_hbm, wq_hbm, wuk_hbm, wuv_hbm, wo_hbm,
            w1_hbm, b1_hbm, w2_hbm, b2_hbm,
            o_ref,
            x_v, ckv_v, wq_v, wuk_v, wuv_v, wo_v, w1_v, b1_v, w2_v, b2_v,
            e_v, et_v, lhs_v, qa_v, m_v, l_v, acc_v, s_v, cb_v, stage,
            sem,
            *, B, S, C, H, D, M, FF, wo_splits):
    n_kv = S // KV_DMA_ROWS
    NHG = H // HG
    G = C // LANES
    R = B * HG
    W = LANES * HG
    n_vpu = len(WO_VPU_TAIL)
    vpu_heads = sum(WO_VPU_TAIL) // D
    KV0 = 8 + len(wo_splits)
    ST0 = KV0 + B * n_kv

    cp_x = pltpu.make_async_copy(x_hbm, x_v, sem.at[0])
    cp_wq = pltpu.make_async_copy(wq_hbm, wq_v, sem.at[1])
    cp_wuk = pltpu.make_async_copy(wuk_hbm, wuk_v, sem.at[2])
    cp_b1 = pltpu.make_async_copy(b1_hbm, b1_v, sem.at[3])
    cp_b2 = pltpu.make_async_copy(b2_hbm, b2_v, sem.at[4])
    cp_w1 = pltpu.make_async_copy(w1_hbm, w1_v, sem.at[5])
    cp_w2 = pltpu.make_async_copy(w2_hbm, w2_v, sem.at[6])
    cp_wuv = pltpu.make_async_copy(wuv_hbm, wuv_v, sem.at[7])
    cp_wo = [
        pltpu.make_async_copy(wo_hbm.at[pl.ds(r0, r1 - r0)],
                              wo_v.at[pl.ds(r0, r1 - r0)], sem.at[8 + k])
        for k, (r0, r1) in enumerate(wo_splits)
    ]

    def kv_copy(b, j):
        rows = pl.ds(j * KV_DMA_ROWS, KV_DMA_ROWS)
        return pltpu.make_async_copy(ckv_hbm.at[b, rows], ckv_v.at[b, rows],
                                     sem.at[KV0 + b * n_kv + j])

    def stage_slot(p):
        return stage.at[pl.ds((p % STAGE_SLOTS) * STAGE_ROWS, STAGE_ROWS)]

    def stage_in(p):
        return pltpu.make_async_copy(wo_hbm.at[pl.ds(p * STAGE_ROWS, STAGE_ROWS)],
                                     stage_slot(p), sem.at[ST0 + 2 * p])

    def stage_out(p):
        return pltpu.make_async_copy(stage_slot(p),
                                     wo_v.at[pl.ds(p * STAGE_ROWS, STAGE_ROWS)],
                                     sem.at[ST0 + 2 * p + 1])

    def stage_step(j):
        if j - 1 < STAGE_PIECES:
            stage_in(j - 1).wait()
            stage_out(j - 1).start()
        if j + 1 < STAGE_PIECES:
            if j + 1 >= STAGE_SLOTS:
                stage_out(j + 1 - STAGE_SLOTS).wait()
            stage_in(j + 1).start()

    cp_x.start()
    cp_wq.start()
    stage_in(0).start()
    stage_in(1).start()
    cp_wuk.start()
    for b in range(B):
        for j in range(n_kv):
            kv_copy(b, j).start()
    cp_b1.start()
    cp_b2.start()
    cp_w1.start()
    cp_w2.start()
    cp_wuv.start()
    for cp in cp_wo:
        cp.start()

    e_v[...] = (lax.broadcasted_iota(jnp.int32, (LANES, W), 0)
                == lax.broadcasted_iota(jnp.int32, (LANES, W), 1) // HG
                ).astype(F32).astype(BF16)
    et_v[...] = (lax.broadcasted_iota(jnp.int32, (W, LANES), 0) // HG
                 == lax.broadcasted_iota(jnp.int32, (W, LANES), 1)
                 ).astype(F32).astype(BF16)

    def diag_mask(rows):
        return (lax.broadcasted_iota(jnp.int32, (rows, W), 0) % HG
                == lax.broadcasted_iota(jnp.int32, (rows, W), 1) % HG)

    def expand(a):
        st = jnp.concatenate([a[:, g * LANES:(g + 1) * LANES] for g in range(G)], axis=0)
        rep = jnp.dot(st, e_v[...], preferred_element_type=F32)
        return jnp.where(diag_mask(G * R), rep, 0.0).astype(BF16)

    def head_group(w_ref, g, hg):
        return w_ref[g * LANES:(g + 1) * LANES, hg * HG:(hg + 1) * HG, :].reshape(W, D)

    cp_x.wait()
    x32 = x_v[...].astype(F32)
    xs = [x32[b:b + 1] for b in range(B)]
    xns = []
    for xb in xs:
        mu = jnp.mean(xb, axis=-1, keepdims=True)
        xc = xb - mu
        var = jnp.mean(xc * xc, axis=-1, keepdims=True)
        xns.append(xc / jnp.sqrt(var + 1e-5))
    xrows = jnp.concatenate(
        [jnp.broadcast_to(xn, (HG, M)) for xn in xns], axis=0).astype(BF16)

    lq = expand(xrows)
    cp_wq.wait()
    stage_step(1)
    scale = D ** -0.5
    qs = []
    for hg in range(NHG):
        acc = jnp.zeros((R, D), F32)
        for g in range(G):
            acc += jnp.dot(lq[g * R:(g + 1) * R], head_group(wq_v, g, hg),
                           preferred_element_type=F32)
        qs.append((acc * scale).astype(BF16))

    cp_wuk.wait()
    stage_step(2)
    dm = diag_mask(R)
    for hg in range(NHG):
        for g in range(G):
            st = lax.dot_general(qs[hg], head_group(wuk_v, g, hg), NT,
                                 preferred_element_type=F32)
            k = hg * G + g
            lhs_v[k * R:(k + 1) * R, :] = jnp.where(dm, st, 0.0).astype(BF16)
    qa = jnp.dot(lhs_v[...], et_v[...], preferred_element_type=F32).astype(BF16)
    for b in range(B):
        for hg in range(NHG):
            for g in range(G):
                r0 = (hg * G + g) * R + b * HG
                qa_v[b, hg * HG:(hg + 1) * HG, g * LANES:(g + 1) * LANES] = qa[r0:r0 + HG]

    m_v[...] = jnp.full(m_v.shape, -jnp.inf, F32)
    l_v[...] = jnp.zeros(l_v.shape, F32)
    acc_v[...] = jnp.zeros(acc_v.shape, F32)
    sub = KV_DMA_ROWS // TK

    def kv_step(t, carry):
        b = t // (S // TK)
        j = t % (S // TK)

        @pl.when(j % sub == 0)
        def _():
            kv_copy(b, j // sub).wait()

        for k in range(B * n_kv):
            pl.when(t == k * sub)(functools.partial(stage_step, 3 + k))

        c = ckv_v[b, pl.ds(pl.multiple_of(j * TK, TK), TK), :]
        s = lax.dot_general(qa_v[b], c, NT, preferred_element_type=F32)
        m_old = m_v[b]
        m_new = jnp.maximum(m_old, jnp.max(s, axis=-1, keepdims=True))
        alpha = jnp.exp(m_old - m_new)
        p = jnp.exp(s - m_new)
        l_v[b] = alpha * l_v[b] + jnp.sum(p, axis=-1, keepdims=True)
        acc_v[b] = alpha * acc_v[b] + jnp.dot(p.astype(BF16), c, preferred_element_type=F32)
        m_v[b] = m_new
        return carry

    lax.fori_loop(0, B * (S // TK), kv_step, 0)

    ctxc = [(acc_v[b] / l_v[b]).astype(BF16) for b in range(B)]
    for hg in range(NHG):
        a = jnp.concatenate([ctxc[b][hg * HG:(hg + 1) * HG] for b in range(B)], axis=0)
        lhs_v[hg * G * R:(hg + 1) * G * R, :] = expand(a)

    cp_b1.wait()
    cp_b2.wait()
    cp_w1.wait()
    hid = jnp.dot(xrows, w1_v[...], preferred_element_type=F32)
    hid = hid + b1_v[...].astype(F32).reshape(1, FF)
    hid = jax.nn.gelu(hid, approximate=True).astype(BF16)
    cp_w2.wait()
    y = jnp.dot(hid, w2_v[...], preferred_element_type=F32)
    y = y + b2_v[...].astype(F32).reshape(1, M)
    s_v[...] = y * jax.nn.sigmoid(y)
    for j in range(3 + B * n_kv, STAGE_PIECES + 1):
        stage_step(j)
    gate = s_v[...]

    cp_wuv.wait()
    ctx = []
    for hg in range(NHG):
        acc = jnp.zeros((R, D), F32)
        for g in range(G):
            k = hg * G + g
            acc += jnp.dot(lhs_v[k * R:(k + 1) * R, :], head_group(wuv_v, g, hg),
                           preferred_element_type=F32)
        ctx.append(acc)

    row_i = lax.broadcasted_iota(jnp.int32, (R, D), 0) % HG
    lo = jnp.concatenate(
        [jnp.where(row_i == h % HG, ctx[h // HG], 0.0).astype(BF16)
         for h in range(H - vpu_heads)], axis=1)
    for b in range(B):
        for u in range(vpu_heads):
            i = b * HG + HG - vpu_heads + u
            row = ctx[NHG - 1][i:i + 1, :].astype(BF16).astype(F32)
            cb_v[b, u * D:(u + 1) * D] = jnp.transpose(jnp.broadcast_to(row, (LANES, D)))

    for p in range(max(STAGE_PIECES - STAGE_SLOTS, 0), STAGE_PIECES):
        stage_out(p).wait()
    r_staged = STAGE_PIECES * STAGE_ROWS
    s_v[...] = jnp.dot(lo[:, :r_staged], wo_v[:r_staged], preferred_element_type=F32)
    n_mxu = len(wo_splits) - n_vpu
    for k in range(n_mxu):
        r0, r1 = wo_splits[k]
        cp_wo[k].wait()
        part = s_v[...] + jnp.dot(lo[:, r0:r1], wo_v[r0:r1], preferred_element_type=F32)
        if k + 1 < n_mxu:
            s_v[...] = part
    for b in range(B):
        s_v[b * SUB:(b + 1) * SUB, :] = (part[b * HG:b * HG + SUB]
                                         + part[b * HG + SUB:(b + 1) * HG])
    v0 = (H - vpu_heads) * D
    for k in range(n_mxu, len(wo_splits)):
        r0, r1 = wo_splits[k]
        cp_wo[k].wait()
        w32 = wo_v[r0:r1].astype(F32)
        accs = []
        for b in range(B):
            cb = cb_v[b, r0 - v0:r1 - v0, :]
            prod = w32 * jnp.concatenate([cb] * (M // LANES), axis=1)
            a = s_v[b * SUB:(b + 1) * SUB, :]
            for u in range((r1 - r0) // SUB):
                a = a + prod[u * SUB:(u + 1) * SUB]
            accs.append(a)
            if k + 1 < len(wo_splits):
                s_v[b * SUB:(b + 1) * SUB, :] = a
    outs = [xs[b] + jnp.sum(accs[b], axis=0, keepdims=True) * gate[b * HG:b * HG + 1]
            for b in range(B)]
    o_ref[...] = jnp.concatenate(outs, axis=0).astype(o_ref.dtype)


def _compiler_params():
    vmem = 100 * 1024 * 1024
    try:
        return pltpu.CompilerParams(vmem_limit_bytes=vmem, disable_semaphore_checks=True)
    except TypeError:
        return pltpu.CompilerParams(vmem_limit_bytes=vmem)


@jax.jit
def pallas_recurrent_scan__compressed_kv_cla__dense_activation_gelu__decode_kernel(
    A_x: jax.Array,
    A_c_kv: jax.Array,
    A_w_q: jax.Array,
    A_w_uk: jax.Array,
    A_w_uv: jax.Array,
    A_w_o: jax.Array,
    B_x: jax.Array,
    B_w1: jax.Array,
    B_b1: jax.Array,
    B_w2: jax.Array,
    B_b2: jax.Array,
):
    del B_x
    B, Sq, M = A_x.shape
    _, S, C = A_c_kv.shape
    _, H, D = A_w_q.shape
    FF = B_w1.shape[1]
    assert Sq == 1 and M == C and D == LANES and H % HG == 0 and S % KV_DMA_ROWS == 0
    assert sum(WO_VPU_TAIL) % D == 0 and sum(WO_VPU_TAIL) <= HG * D
    G = C // LANES
    R = B * HG
    W = LANES * HG

    r = STAGE_PIECES * STAGE_ROWS
    sizes = (H * D - r - sum(WO_MXU_TAIL) - sum(WO_VPU_TAIL),) + WO_MXU_TAIL + WO_VPU_TAIL
    wo_splits = []
    for n in sizes:
        wo_splits.append((r, r + n))
        r += n
    n_sem = 8 + len(wo_splits) + B * (S // KV_DMA_ROWS) + 2 * STAGE_PIECES

    kernel = functools.partial(_kernel, B=B, S=S, C=C, H=H, D=D, M=M, FF=FF,
                               wo_splits=tuple(wo_splits))
    hbm = pl.BlockSpec(memory_space=pl.ANY)
    out = pl.pallas_call(
        kernel,
        out_shape=jax.ShapeDtypeStruct((B, M), A_x.dtype),
        in_specs=[hbm] * 10,
        out_specs=pl.BlockSpec(memory_space=pltpu.VMEM),
        scratch_shapes=[
            pltpu.VMEM((B, M), BF16),
            pltpu.VMEM(A_c_kv.shape, BF16),
            pltpu.VMEM(A_w_q.shape, BF16),
            pltpu.VMEM(A_w_uk.shape, BF16),
            pltpu.VMEM(A_w_uv.shape, BF16),
            pltpu.VMEM((H * D, M), BF16),
            pltpu.VMEM(B_w1.shape, BF16),
            pltpu.VMEM(B_b1.shape, BF16),
            pltpu.VMEM(B_w2.shape, BF16),
            pltpu.VMEM(B_b2.shape, BF16),
            pltpu.VMEM((LANES, W), BF16),
            pltpu.VMEM((W, LANES), BF16),
            pltpu.VMEM(((H // HG) * G * R, W), BF16),
            pltpu.VMEM((B, H, C), BF16),
            pltpu.VMEM((B, H, 1), F32),
            pltpu.VMEM((B, H, 1), F32),
            pltpu.VMEM((B, H, C), F32),
            pltpu.VMEM((R, M), F32),
            pltpu.VMEM((B, sum(WO_VPU_TAIL), LANES), F32),
            pltpu.SMEM((STAGE_SLOTS * STAGE_ROWS, M), BF16),
            pltpu.SemaphoreType.DMA((n_sem,)),
        ],
        compiler_params=_compiler_params(),
    )(A_x.reshape(B, M), A_c_kv, A_w_q, A_w_uk, A_w_uv, A_w_o.reshape(H * D, M),
      B_w1, B_b1, B_w2, B_b2)
    return out.reshape(B, Sq, M)
```

```python
import functools

import jax
import jax.numpy as jnp
from jax import lax
import jax.experimental.pallas as pl
import jax.experimental.pallas.tpu as pltpu

F32 = jnp.float32
BF16 = jnp.bfloat16

LANES = 128
SUB = 8
HG = 16
TK = 2048
KV_DMA_ROWS = 4096
STAGE_ROWS = 144
STAGE_PIECES = 11
STAGE_SLOTS = 4
WO_MXU_TAIL = (512,)
WO_VPU_TAIL = (128, 96, 32)
NT = (((1,), (1,)), ((), ()))


def _kernel(x_hbm, ckv_hbm, wq_hbm, wuk_hbm, wuv_hbm, wo_hbm,
            w1_hbm, b1_hbm, w2_hbm, b2_hbm,
            o_ref,
            x_v, ckv_v, wq_v, wuk_v, wuv_v, wo_v, w1_v, b1_v, w2_v, b2_v,
            e_v, et_v, lhs_v, qa_v, m_v, l_v, acc_v, s_v, cb_v, stage,
            sem,
            *, B, S, C, H, D, M, FF, wo_splits):
    n_kv = S // KV_DMA_ROWS
    NHG = H // HG
    G = C // LANES
    R = B * HG
    W = LANES * HG
    n_vpu = len(WO_VPU_TAIL)
    vpu_heads = sum(WO_VPU_TAIL) // D
    KV0 = 8 + len(wo_splits)
    ST0 = KV0 + B * n_kv

    cp_x = pltpu.make_async_copy(x_hbm, x_v, sem.at[0])
    cp_wq = pltpu.make_async_copy(wq_hbm, wq_v, sem.at[1])
    cp_wuk = pltpu.make_async_copy(wuk_hbm, wuk_v, sem.at[2])
    cp_b1 = pltpu.make_async_copy(b1_hbm, b1_v, sem.at[3])
    cp_b2 = pltpu.make_async_copy(b2_hbm, b2_v, sem.at[4])
    cp_w1 = pltpu.make_async_copy(w1_hbm, w1_v, sem.at[5])
    cp_w2 = pltpu.make_async_copy(w2_hbm, w2_v, sem.at[6])
    cp_wuv = pltpu.make_async_copy(wuv_hbm, wuv_v, sem.at[7])
    cp_wo = [
        pltpu.make_async_copy(wo_hbm.at[pl.ds(r0, r1 - r0)],
                              wo_v.at[pl.ds(r0, r1 - r0)], sem.at[8 + k])
        for k, (r0, r1) in enumerate(wo_splits)
    ]

    def kv_copy(b, j):
        rows = pl.ds(j * KV_DMA_ROWS, KV_DMA_ROWS)
        return pltpu.make_async_copy(ckv_hbm.at[b, rows], ckv_v.at[b, rows],
                                     sem.at[KV0 + b * n_kv + j])

    def stage_slot(p):
        return stage.at[pl.ds((p % STAGE_SLOTS) * STAGE_ROWS, STAGE_ROWS)]

    def stage_in(p):
        return pltpu.make_async_copy(wo_hbm.at[pl.ds(p * STAGE_ROWS, STAGE_ROWS)],
                                     stage_slot(p), sem.at[ST0 + 2 * p])

    def stage_out(p):
        return pltpu.make_async_copy(stage_slot(p),
                                     wo_v.at[pl.ds(p * STAGE_ROWS, STAGE_ROWS)],
                                     sem.at[ST0 + 2 * p + 1])

    def stage_step(j):
        if j - 1 < STAGE_PIECES:
            stage_in(j - 1).wait()
            stage_out(j - 1).start()
        if j + 1 < STAGE_PIECES:
            if j + 1 >= STAGE_SLOTS:
                stage_out(j + 1 - STAGE_SLOTS).wait()
            stage_in(j + 1).start()

    cp_x.start()
    cp_wq.start()
    stage_in(0).start()
    stage_in(1).start()
    cp_wuk.start()
    for b in range(B):
        for j in range(n_kv):
            kv_copy(b, j).start()
    cp_b1.start()
    cp_b2.start()
    cp_w1.start()
    cp_w2.start()
    cp_wuv.start()
    for cp in cp_wo:
        cp.start()

    e_v[...] = (lax.broadcasted_iota(jnp.int32, (LANES, W), 0)
                == lax.broadcasted_iota(jnp.int32, (LANES, W), 1) // HG
                ).astype(F32).astype(BF16)
    et_v[...] = (lax.broadcasted_iota(jnp.int32, (W, LANES), 0) // HG
                 == lax.broadcasted_iota(jnp.int32, (W, LANES), 1)
                 ).astype(F32).astype(BF16)

    def diag_mask(rows):
        return (lax.broadcasted_iota(jnp.int32, (rows, W), 0) % HG
                == lax.broadcasted_iota(jnp.int32, (rows, W), 1) % HG)

    def expand(a):
        st = jnp.concatenate([a[:, g * LANES:(g + 1) * LANES] for g in range(G)], axis=0)
        rep = jnp.dot(st, e_v[...], preferred_element_type=F32)
        return jnp.where(diag_mask(G * R), rep, 0.0).astype(BF16)

    def head_group(w_ref, g, hg):
        return w_ref[g * LANES:(g + 1) * LANES, hg * HG:(hg + 1) * HG, :].reshape(W, D)

    cp_x.wait()
    x32 = x_v[...].astype(F32)
    xs = [x32[b:b + 1] for b in range(B)]
    xns = []
    for xb in xs:
        mu = jnp.mean(xb, axis=-1, keepdims=True)
        xc = xb - mu
        var = jnp.mean(xc * xc, axis=-1, keepdims=True)
        xns.append(xc / jnp.sqrt(var + 1e-5))
    xrows = jnp.concatenate(
        [jnp.broadcast_to(xn, (HG, M)) for xn in xns], axis=0).astype(BF16)

    lq = expand(xrows)
    cp_wq.wait()
    stage_step(1)
    scale = D ** -0.5
    qs = []
    for hg in range(NHG):
        acc = jnp.zeros((R, D), F32)
        for g in range(G):
            acc += jnp.dot(lq[g * R:(g + 1) * R], head_group(wq_v, g, hg),
                           preferred_element_type=F32)
        qs.append((acc * scale).astype(BF16))

    cp_wuk.wait()
    stage_step(2)
    dm = diag_mask(R)
    for hg in range(NHG):
        for g in range(G):
            st = lax.dot_general(qs[hg], head_group(wuk_v, g, hg), NT,
                                 preferred_element_type=F32)
            k = hg * G + g
            lhs_v[k * R:(k + 1) * R, :] = jnp.where(dm, st, 0.0).astype(BF16)
    qa = jnp.dot(lhs_v[...], et_v[...], preferred_element_type=F32).astype(BF16)
    for b in range(B):
        for hg in range(NHG):
            for g in range(G):
                r0 = (hg * G + g) * R + b * HG
                qa_v[b, hg * HG:(hg + 1) * HG, g * LANES:(g + 1) * LANES] = qa[r0:r0 + HG]

    m_v[...] = jnp.full(m_v.shape, -jnp.inf, F32)
    l_v[...] = jnp.zeros(l_v.shape, F32)
    acc_v[...] = jnp.zeros(acc_v.shape, F32)
    sub = KV_DMA_ROWS // TK

    def kv_step(t, carry):
        b = t // (S // TK)
        j = t % (S // TK)

        @pl.when(j % sub == 0)
        def _():
            kv_copy(b, j // sub).wait()

        for k in range(B * n_kv):
            pl.when(t == k * sub)(functools.partial(stage_step, 3 + k))

        c = ckv_v[b, pl.ds(pl.multiple_of(j * TK, TK), TK), :]
        s = lax.dot_general(qa_v[b], c, NT, preferred_element_type=F32)
        m_old = m_v[b]
        m_new = jnp.maximum(m_old, jnp.max(s, axis=-1, keepdims=True))
        alpha = jnp.exp(m_old - m_new)
        p = jnp.exp(s - m_new)
        l_v[b] = alpha * l_v[b] + jnp.sum(p, axis=-1, keepdims=True)
        acc_v[b] = alpha * acc_v[b] + jnp.dot(p.astype(BF16), c, preferred_element_type=F32)
        m_v[b] = m_new
        return carry

    lax.fori_loop(0, B * (S // TK), kv_step, 0)

    ctxc = [(acc_v[b] / l_v[b]).astype(BF16) for b in range(B)]
    for hg in range(NHG):
        a = jnp.concatenate([ctxc[b][hg * HG:(hg + 1) * HG] for b in range(B)], axis=0)
        lhs_v[hg * G * R:(hg + 1) * G * R, :] = expand(a)

    cp_b1.wait()
    cp_b2.wait()
    cp_w1.wait()
    hid = jnp.dot(xrows, w1_v[...], preferred_element_type=F32)
    hid = hid + b1_v[...].astype(F32).reshape(1, FF)
    hid = jax.nn.gelu(hid, approximate=True).astype(BF16)
    cp_w2.wait()
    y = jnp.dot(hid, w2_v[...], preferred_element_type=F32)
    y = y + b2_v[...].astype(F32).reshape(1, M)
    s_v[...] = y * jax.nn.sigmoid(y)
    for j in range(3 + B * n_kv, STAGE_PIECES + 1):
        stage_step(j)
    gate = s_v[...]

    cp_wuv.wait()
    ctx = []
    for hg in range(NHG):
        acc = jnp.zeros((R, D), F32)
        for g in range(G):
            k = hg * G + g
            acc += jnp.dot(lhs_v[k * R:(k + 1) * R, :], head_group(wuv_v, g, hg),
                           preferred_element_type=F32)
        ctx.append(acc)

    row_i = lax.broadcasted_iota(jnp.int32, (R, D), 0) % HG
    lo = jnp.concatenate(
        [jnp.where(row_i == h % HG, ctx[h // HG], 0.0).astype(BF16)
         for h in range(H - vpu_heads)], axis=1)
    for b in range(B):
        for u in range(vpu_heads):
            i = b * HG + HG - vpu_heads + u
            row = ctx[NHG - 1][i:i + 1, :].astype(BF16).astype(F32)
            cb_v[b, u * D:(u + 1) * D] = jnp.transpose(jnp.broadcast_to(row, (LANES, D)))

    for p in range(max(STAGE_PIECES - STAGE_SLOTS, 0), STAGE_PIECES):
        stage_out(p).wait()
    r_staged = STAGE_PIECES * STAGE_ROWS
    s_v[...] = jnp.dot(lo[:, :r_staged], wo_v[:r_staged], preferred_element_type=F32)
    n_mxu = len(wo_splits) - n_vpu
    for k in range(n_mxu):
        r0, r1 = wo_splits[k]
        cp_wo[k].wait()
        part = s_v[...] + jnp.dot(lo[:, r0:r1], wo_v[r0:r1], preferred_element_type=F32)
        if k + 1 < n_mxu:
            s_v[...] = part
    for b in range(B):
        s_v[b * SUB:(b + 1) * SUB, :] = (part[b * HG:b * HG + SUB]
                                         + part[b * HG + SUB:(b + 1) * HG])
    v0 = (H - vpu_heads) * D
    for k in range(n_mxu, len(wo_splits)):
        r0, r1 = wo_splits[k]
        cp_wo[k].wait()
        accs = [s_v[b * SUB:(b + 1) * SUB, :] for b in range(B)]
        for r in range(r0, r1, HG):
            w32 = wo_v[r:r + HG].astype(F32)
            for b in range(B):
                cb = cb_v[b, r - v0:r - v0 + HG, :]
                prod = w32 * jnp.concatenate([cb] * (M // LANES), axis=1)
                accs[b] = accs[b] + prod[:SUB] + prod[SUB:]
        if k + 1 < len(wo_splits):
            for b in range(B):
                s_v[b * SUB:(b + 1) * SUB, :] = accs[b]
    outs = [xs[b] + jnp.sum(accs[b], axis=0, keepdims=True) * gate[b * HG:b * HG + 1]
            for b in range(B)]
    o_ref[...] = jnp.concatenate(outs, axis=0).astype(o_ref.dtype)


def _compiler_params():
    vmem = 100 * 1024 * 1024
    try:
        return pltpu.CompilerParams(vmem_limit_bytes=vmem, disable_semaphore_checks=True)
    except TypeError:
        return pltpu.CompilerParams(vmem_limit_bytes=vmem)


@jax.jit
def pallas_recurrent_scan__compressed_kv_cla__dense_activation_gelu__decode_kernel(
    A_x: jax.Array,
    A_c_kv: jax.Array,
    A_w_q: jax.Array,
    A_w_uk: jax.Array,
    A_w_uv: jax.Array,
    A_w_o: jax.Array,
    B_x: jax.Array,
    B_w1: jax.Array,
    B_b1: jax.Array,
    B_w2: jax.Array,
    B_b2: jax.Array,
):
    del B_x
    B, Sq, M = A_x.shape
    _, S, C = A_c_kv.shape
    _, H, D = A_w_q.shape
    FF = B_w1.shape[1]
    assert Sq == 1 and M == C and D == LANES and H % HG == 0 and S % KV_DMA_ROWS == 0
    assert sum(WO_VPU_TAIL) % D == 0 and sum(WO_VPU_TAIL) <= HG * D
    G = C // LANES
    R = B * HG
    W = LANES * HG

    r = STAGE_PIECES * STAGE_ROWS
    sizes = (H * D - r - sum(WO_MXU_TAIL) - sum(WO_VPU_TAIL),) + WO_MXU_TAIL + WO_VPU_TAIL
    wo_splits = []
    for n in sizes:
        wo_splits.append((r, r + n))
        r += n
    n_sem = 8 + len(wo_splits) + B * (S // KV_DMA_ROWS) + 2 * STAGE_PIECES

    kernel = functools.partial(_kernel, B=B, S=S, C=C, H=H, D=D, M=M, FF=FF,
                               wo_splits=tuple(wo_splits))
    hbm = pl.BlockSpec(memory_space=pl.ANY)
    out = pl.pallas_call(
        kernel,
        out_shape=jax.ShapeDtypeStruct((B, M), A_x.dtype),
        in_specs=[hbm] * 10,
        out_specs=pl.BlockSpec(memory_space=pltpu.VMEM),
        scratch_shapes=[
            pltpu.VMEM((B, M), BF16),
            pltpu.VMEM(A_c_kv.shape, BF16),
            pltpu.VMEM(A_w_q.shape, BF16),
            pltpu.VMEM(A_w_uk.shape, BF16),
            pltpu.VMEM(A_w_uv.shape, BF16),
            pltpu.VMEM((H * D, M), BF16),
            pltpu.VMEM(B_w1.shape, BF16),
            pltpu.VMEM(B_b1.shape, BF16),
            pltpu.VMEM(B_w2.shape, BF16),
            pltpu.VMEM(B_b2.shape, BF16),
            pltpu.VMEM((LANES, W), BF16),
            pltpu.VMEM((W, LANES), BF16),
            pltpu.VMEM(((H // HG) * G * R, W), BF16),
            pltpu.VMEM((B, H, C), BF16),
            pltpu.VMEM((B, H, 1), F32),
            pltpu.VMEM((B, H, 1), F32),
            pltpu.VMEM((B, H, C), F32),
            pltpu.VMEM((R, M), F32),
            pltpu.VMEM((B, sum(WO_VPU_TAIL), LANES), F32),
            pltpu.SMEM((STAGE_SLOTS * STAGE_ROWS, M), BF16),
            pltpu.SemaphoreType.DMA((n_sem,)),
        ],
        compiler_params=_compiler_params(),
    )(A_x.reshape(B, M), A_c_kv, A_w_q, A_w_uk, A_w_uv, A_w_o.reshape(H * D, M),
      B_w1, B_b1, B_w2, B_b2)
    return out.reshape(B, Sq, M)
```

```python
import functools

import jax
import jax.numpy as jnp
from jax import lax
import jax.experimental.pallas as pl
import jax.experimental.pallas.tpu as pltpu

F32 = jnp.float32
BF16 = jnp.bfloat16

LANES = 128
SUB = 8
HG = 16
TK = 2048
KV_DMA_ROWS = 4096
STAGE_ROWS = 144
STAGE_PIECES = 11
STAGE_SLOTS = 4
WO_MXU_TAIL = (512,)
WO_VPU_TAIL = (128, 96, 32)
NT = (((1,), (1,)), ((), ()))


def _kernel(x_hbm, ckv_hbm, wq_hbm, wuk_hbm, wuv_hbm, wo_hbm,
            w1_hbm, b1_hbm, w2_hbm, b2_hbm,
            o_ref,
            x_v, ckv_v, wq_v, wuk_v, wuv_v, wo_v, w1_v, b1_v, w2_v, b2_v,
            e_v, et_v, lhs_v, qa_v, m_v, l_v, acc_v, s_v, fin_v, cb_v, stage,
            sem,
            *, B, S, C, H, D, M, FF, wo_splits):
    n_kv = S // KV_DMA_ROWS
    NHG = H // HG
    G = C // LANES
    R = B * HG
    W = LANES * HG
    n_vpu = len(WO_VPU_TAIL)
    vpu_heads = sum(WO_VPU_TAIL) // D
    KV0 = 8 + len(wo_splits)
    ST0 = KV0 + B * n_kv

    cp_x = pltpu.make_async_copy(x_hbm, x_v, sem.at[0])
    cp_wq = pltpu.make_async_copy(wq_hbm, wq_v, sem.at[1])
    cp_wuk = pltpu.make_async_copy(wuk_hbm, wuk_v, sem.at[2])
    cp_b1 = pltpu.make_async_copy(b1_hbm, b1_v, sem.at[3])
    cp_b2 = pltpu.make_async_copy(b2_hbm, b2_v, sem.at[4])
    cp_w1 = pltpu.make_async_copy(w1_hbm, w1_v, sem.at[5])
    cp_w2 = pltpu.make_async_copy(w2_hbm, w2_v, sem.at[6])
    cp_wuv = pltpu.make_async_copy(wuv_hbm, wuv_v, sem.at[7])
    cp_wo = [
        pltpu.make_async_copy(wo_hbm.at[pl.ds(r0, r1 - r0)],
                              wo_v.at[pl.ds(r0, r1 - r0)], sem.at[8 + k])
        for k, (r0, r1) in enumerate(wo_splits)
    ]

    def kv_copy(b, j):
        rows = pl.ds(j * KV_DMA_ROWS, KV_DMA_ROWS)
        return pltpu.make_async_copy(ckv_hbm.at[b, rows], ckv_v.at[b, rows],
                                     sem.at[KV0 + b * n_kv + j])

    def stage_slot(p):
        return stage.at[pl.ds((p % STAGE_SLOTS) * STAGE_ROWS, STAGE_ROWS)]

    def stage_in(p):
        return pltpu.make_async_copy(wo_hbm.at[pl.ds(p * STAGE_ROWS, STAGE_ROWS)],
                                     stage_slot(p), sem.at[ST0 + 2 * p])

    def stage_out(p):
        return pltpu.make_async_copy(stage_slot(p),
                                     wo_v.at[pl.ds(p * STAGE_ROWS, STAGE_ROWS)],
                                     sem.at[ST0 + 2 * p + 1])

    def stage_step(j):
        if j - 1 < STAGE_PIECES:
            stage_in(j - 1).wait()
            stage_out(j - 1).start()
        if j + 1 < STAGE_PIECES:
            if j + 1 >= STAGE_SLOTS:
                stage_out(j + 1 - STAGE_SLOTS).wait()
            stage_in(j + 1).start()

    cp_x.start()
    cp_wq.start()
    stage_in(0).start()
    stage_in(1).start()
    cp_wuk.start()
    for b in range(B):
        for j in range(n_kv):
            kv_copy(b, j).start()
    cp_b1.start()
    cp_b2.start()
    cp_w1.start()
    cp_w2.start()
    cp_wuv.start()
    for cp in cp_wo:
        cp.start()

    e_v[...] = (lax.broadcasted_iota(jnp.int32, (LANES, W), 0)
                == lax.broadcasted_iota(jnp.int32, (LANES, W), 1) // HG
                ).astype(F32).astype(BF16)
    et_v[...] = (lax.broadcasted_iota(jnp.int32, (W, LANES), 0) // HG
                 == lax.broadcasted_iota(jnp.int32, (W, LANES), 1)
                 ).astype(F32).astype(BF16)

    def diag_mask(rows):
        return (lax.broadcasted_iota(jnp.int32, (rows, W), 0) % HG
                == lax.broadcasted_iota(jnp.int32, (rows, W), 1) % HG)

    def expand(a):
        st = jnp.concatenate([a[:, g * LANES:(g + 1) * LANES] for g in range(G)], axis=0)
        rep = jnp.dot(st, e_v[...], preferred_element_type=F32)
        return jnp.where(diag_mask(G * R), rep, 0.0).astype(BF16)

    def head_group(w_ref, g, hg):
        return w_ref[g * LANES:(g + 1) * LANES, hg * HG:(hg + 1) * HG, :].reshape(W, D)

    cp_x.wait()
    x32 = x_v[...].astype(F32)
    xs = [x32[b:b + 1] for b in range(B)]
    xns = []
    for xb in xs:
        mu = jnp.mean(xb, axis=-1, keepdims=True)
        xc = xb - mu
        var = jnp.mean(xc * xc, axis=-1, keepdims=True)
        xns.append(xc / jnp.sqrt(var + 1e-5))
    xrows = jnp.concatenate(
        [jnp.broadcast_to(xn, (HG, M)) for xn in xns], axis=0).astype(BF16)

    lq = expand(xrows)
    cp_wq.wait()
    stage_step(1)
    scale = D ** -0.5
    qs = []
    for hg in range(NHG):
        acc = jnp.zeros((R, D), F32)
        for g in range(G):
            acc += jnp.dot(lq[g * R:(g + 1) * R], head_group(wq_v, g, hg),
                           preferred_element_type=F32)
        qs.append((acc * scale).astype(BF16))

    cp_wuk.wait()
    stage_step(2)
    dm = diag_mask(R)
    for hg in range(NHG):
        for g in range(G):
            st = lax.dot_general(qs[hg], head_group(wuk_v, g, hg), NT,
                                 preferred_element_type=F32)
            k = hg * G + g
            lhs_v[k * R:(k + 1) * R, :] = jnp.where(dm, st, 0.0).astype(BF16)
    qa = jnp.dot(lhs_v[...], et_v[...], preferred_element_type=F32).astype(BF16)
    for b in range(B):
        for hg in range(NHG):
            for g in range(G):
                r0 = (hg * G + g) * R + b * HG
                qa_v[b, hg * HG:(hg + 1) * HG, g * LANES:(g + 1) * LANES] = qa[r0:r0 + HG]

    m_v[...] = jnp.full(m_v.shape, -jnp.inf, F32)
    l_v[...] = jnp.zeros(l_v.shape, F32)
    acc_v[...] = jnp.zeros(acc_v.shape, F32)
    sub = KV_DMA_ROWS // TK

    def kv_step(t, carry):
        b = t // (S // TK)
        j = t % (S // TK)

        @pl.when(j % sub == 0)
        def _():
            kv_copy(b, j // sub).wait()

        for k in range(B * n_kv):
            pl.when(t == k * sub)(functools.partial(stage_step, 3 + k))

        c = ckv_v[b, pl.ds(pl.multiple_of(j * TK, TK), TK), :]
        s = lax.dot_general(qa_v[b], c, NT, preferred_element_type=F32)
        m_old = m_v[b]
        m_new = jnp.maximum(m_old, jnp.max(s, axis=-1, keepdims=True))
        alpha = jnp.exp(m_old - m_new)
        p = jnp.exp(s - m_new)
        l_v[b] = alpha * l_v[b] + jnp.sum(p, axis=-1, keepdims=True)
        acc_v[b] = alpha * acc_v[b] + jnp.dot(p.astype(BF16), c, preferred_element_type=F32)
        m_v[b] = m_new
        return carry

    lax.fori_loop(0, B * (S // TK), kv_step, 0)

    ctxc = [(acc_v[b] / l_v[b]).astype(BF16) for b in range(B)]
    for hg in range(NHG):
        a = jnp.concatenate([ctxc[b][hg * HG:(hg + 1) * HG] for b in range(B)], axis=0)
        lhs_v[hg * G * R:(hg + 1) * G * R, :] = expand(a)

    cp_b1.wait()
    cp_b2.wait()
    cp_w1.wait()
    hid = jnp.dot(xrows, w1_v[...], preferred_element_type=F32)
    hid = hid + b1_v[...].astype(F32).reshape(1, FF)
    hid = jax.nn.gelu(hid, approximate=True).astype(BF16)
    cp_w2.wait()
    y = jnp.dot(hid, w2_v[...], preferred_element_type=F32)
    y = y + b2_v[...].astype(F32).reshape(1, M)
    gate = y * jax.nn.sigmoid(y)
    even = lax.broadcasted_iota(jnp.int32, (SUB, M), 0) % 2 == 0
    fin_v[0] = jnp.where(even, gate[:SUB], gate[HG:HG + SUB])
    fin_v[1] = jnp.where(even, jnp.broadcast_to(xs[0], (SUB, M)),
                         jnp.broadcast_to(xs[1], (SUB, M)))
    for j in range(3 + B * n_kv, STAGE_PIECES + 1):
        stage_step(j)

    cp_wuv.wait()
    ctx = []
    for hg in range(NHG):
        acc = jnp.zeros((R, D), F32)
        for g in range(G):
            k = hg * G + g
            acc += jnp.dot(lhs_v[k * R:(k + 1) * R, :], head_group(wuv_v, g, hg),
                           preferred_element_type=F32)
        ctx.append(acc)

    row_i = lax.broadcasted_iota(jnp.int32, (R, D), 0) % HG
    lo = jnp.concatenate(
        [jnp.where(row_i == h % HG, ctx[h // HG], 0.0).astype(BF16)
         for h in range(H - vpu_heads)], axis=1)
    for b in range(B):
        for u in range(vpu_heads):
            i = b * HG + HG - vpu_heads + u
            row = ctx[NHG - 1][i:i + 1, :].astype(BF16).astype(F32)
            cb_v[b, u * D:(u + 1) * D] = jnp.transpose(jnp.broadcast_to(row, (LANES, D)))

    for p in range(max(STAGE_PIECES - STAGE_SLOTS, 0), STAGE_PIECES):
        stage_out(p).wait()
    r_staged = STAGE_PIECES * STAGE_ROWS
    s_v[...] = jnp.dot(lo[:, :r_staged], wo_v[:r_staged], preferred_element_type=F32)
    n_mxu = len(wo_splits) - n_vpu
    for k in range(n_mxu):
        r0, r1 = wo_splits[k]
        cp_wo[k].wait()
        part = s_v[...] + jnp.dot(lo[:, r0:r1], wo_v[r0:r1], preferred_element_type=F32)
        if k + 1 < n_mxu:
            s_v[...] = part
    for b in range(B):
        s_v[b * SUB:(b + 1) * SUB, :] = (part[b * HG:b * HG + SUB]
                                         + part[b * HG + SUB:(b + 1) * HG])
    v0 = (H - vpu_heads) * D
    for k in range(n_mxu, len(wo_splits)):
        r0, r1 = wo_splits[k]
        cp_wo[k].wait()
        accs = [s_v[b * SUB:(b + 1) * SUB, :] for b in range(B)]
        for r in range(r0, r1, HG):
            w32 = wo_v[r:r + HG].astype(F32)
            for b in range(B):
                cb = cb_v[b, r - v0:r - v0 + HG, :]
                prod = w32 * jnp.concatenate([cb] * (M // LANES), axis=1)
                accs[b] = accs[b] + prod[:SUB] + prod[SUB:]
        if k + 1 < len(wo_splits):
            for b in range(B):
                s_v[b * SUB:(b + 1) * SUB, :] = accs[b]
    u = (jnp.where(even, accs[0], accs[1])
         + pltpu.roll(jnp.where(even, accs[1], accs[0]), SUB - 1, axis=0))
    u = u + pltpu.roll(u, 2, axis=0)
    u = u + pltpu.roll(u, 4, axis=0)
    o_ref[...] = (fin_v[1] + u * fin_v[0])[:B].astype(o_ref.dtype)


def _compiler_params():
    vmem = 100 * 1024 * 1024
    try:
        return pltpu.CompilerParams(vmem_limit_bytes=vmem, disable_semaphore_checks=True)
    except TypeError:
        return pltpu.CompilerParams(vmem_limit_bytes=vmem)


@jax.jit
def pallas_recurrent_scan__compressed_kv_cla__dense_activation_gelu__decode_kernel(
    A_x: jax.Array,
    A_c_kv: jax.Array,
    A_w_q: jax.Array,
    A_w_uk: jax.Array,
    A_w_uv: jax.Array,
    A_w_o: jax.Array,
    B_x: jax.Array,
    B_w1: jax.Array,
    B_b1: jax.Array,
    B_w2: jax.Array,
    B_b2: jax.Array,
):
    del B_x
    B, Sq, M = A_x.shape
    _, S, C = A_c_kv.shape
    _, H, D = A_w_q.shape
    FF = B_w1.shape[1]
    assert B == 2 and Sq == 1 and M == C and D == LANES and H % HG == 0 and S % KV_DMA_ROWS == 0
    assert sum(WO_VPU_TAIL) % D == 0 and sum(WO_VPU_TAIL) <= HG * D
    G = C // LANES
    R = B * HG
    W = LANES * HG

    r = STAGE_PIECES * STAGE_ROWS
    sizes = (H * D - r - sum(WO_MXU_TAIL) - sum(WO_VPU_TAIL),) + WO_MXU_TAIL + WO_VPU_TAIL
    wo_splits = []
    for n in sizes:
        wo_splits.append((r, r + n))
        r += n
    n_sem = 8 + len(wo_splits) + B * (S // KV_DMA_ROWS) + 2 * STAGE_PIECES

    kernel = functools.partial(_kernel, B=B, S=S, C=C, H=H, D=D, M=M, FF=FF,
                               wo_splits=tuple(wo_splits))
    hbm = pl.BlockSpec(memory_space=pl.ANY)
    out = pl.pallas_call(
        kernel,
        out_shape=jax.ShapeDtypeStruct((B, M), A_x.dtype),
        in_specs=[hbm] * 10,
        out_specs=pl.BlockSpec(memory_space=pltpu.VMEM),
        scratch_shapes=[
            pltpu.VMEM((B, M), BF16),
            pltpu.VMEM(A_c_kv.shape, BF16),
            pltpu.VMEM(A_w_q.shape, BF16),
            pltpu.VMEM(A_w_uk.shape, BF16),
            pltpu.VMEM(A_w_uv.shape, BF16),
            pltpu.VMEM((H * D, M), BF16),
            pltpu.VMEM(B_w1.shape, BF16),
            pltpu.VMEM(B_b1.shape, BF16),
            pltpu.VMEM(B_w2.shape, BF16),
            pltpu.VMEM(B_b2.shape, BF16),
            pltpu.VMEM((LANES, W), BF16),
            pltpu.VMEM((W, LANES), BF16),
            pltpu.VMEM(((H // HG) * G * R, W), BF16),
            pltpu.VMEM((B, H, C), BF16),
            pltpu.VMEM((B, H, 1), F32),
            pltpu.VMEM((B, H, 1), F32),
            pltpu.VMEM((B, H, C), F32),
            pltpu.VMEM((R, M), F32),
            pltpu.VMEM((2, SUB, M), F32),
            pltpu.VMEM((B, sum(WO_VPU_TAIL), LANES), F32),
            pltpu.SMEM((STAGE_SLOTS * STAGE_ROWS, M), BF16),
            pltpu.SemaphoreType.DMA((n_sem,)),
        ],
        compiler_params=_compiler_params(),
    )(A_x.reshape(B, M), A_c_kv, A_w_q, A_w_uk, A_w_uv, A_w_o.reshape(H * D, M),
      B_w1, B_b1, B_w2, B_b2)
    return out.reshape(B, Sq, M)
```

```python
import functools

import jax
import jax.numpy as jnp
from jax import lax
import jax.experimental.pallas as pl
import jax.experimental.pallas.tpu as pltpu

F32 = jnp.float32
BF16 = jnp.bfloat16

LANES = 128
SUB = 8
HG = 16
TK = 2048
KV_DMA_ROWS = 4096
STAGE_ROWS = 144
STAGE_PIECES = 11
STAGE_SLOTS = 4
WO_MXU_TAIL = (512,)
WO_VPU_TAIL = (128, 96, 32)
NT = (((1,), (1,)), ((), ()))


def _kernel(x_hbm, ckv_hbm, wq_hbm, wuk_hbm, wuv_hbm, wo_hbm,
            w1_hbm, b1_hbm, w2_hbm, b2_hbm,
            o_ref,
            x_v, ckv_v, wq_v, wuk_v, wuv_v, wo_v, w1_v, b1_v, w2_v, b2_v,
            e_v, et_v, lhs_v, qa_v, m_v, l_v, acc_v, s_v, fin_v, cb_v, stage,
            sem,
            *, B, S, C, H, D, M, FF, wo_splits):
    n_kv = S // KV_DMA_ROWS
    NHG = H // HG
    G = C // LANES
    R = B * HG
    W = LANES * HG
    n_vpu = len(WO_VPU_TAIL)
    vpu_heads = sum(WO_VPU_TAIL) // D
    KV0 = 8 + len(wo_splits)
    ST0 = KV0 + B * n_kv

    cp_x = pltpu.make_async_copy(x_hbm, x_v, sem.at[0])
    cp_wq = pltpu.make_async_copy(wq_hbm, wq_v, sem.at[1])
    cp_wuk = pltpu.make_async_copy(wuk_hbm, wuk_v, sem.at[2])
    cp_b1 = pltpu.make_async_copy(b1_hbm, b1_v, sem.at[3])
    cp_b2 = pltpu.make_async_copy(b2_hbm, b2_v, sem.at[4])
    cp_w1 = pltpu.make_async_copy(w1_hbm, w1_v, sem.at[5])
    cp_w2 = pltpu.make_async_copy(w2_hbm, w2_v, sem.at[6])
    cp_wuv = pltpu.make_async_copy(wuv_hbm, wuv_v, sem.at[7])
    cp_wo = [
        pltpu.make_async_copy(wo_hbm.at[pl.ds(r0, r1 - r0)],
                              wo_v.at[pl.ds(r0, r1 - r0)], sem.at[8 + k])
        for k, (r0, r1) in enumerate(wo_splits)
    ]

    def kv_copy(b, j):
        rows = pl.ds(j * KV_DMA_ROWS, KV_DMA_ROWS)
        return pltpu.make_async_copy(ckv_hbm.at[b, rows], ckv_v.at[b, rows],
                                     sem.at[KV0 + b * n_kv + j])

    def stage_slot(p):
        return stage.at[pl.ds((p % STAGE_SLOTS) * STAGE_ROWS, STAGE_ROWS)]

    def stage_in(p):
        return pltpu.make_async_copy(wo_hbm.at[pl.ds(p * STAGE_ROWS, STAGE_ROWS)],
                                     stage_slot(p), sem.at[ST0 + 2 * p])

    def stage_out(p):
        return pltpu.make_async_copy(stage_slot(p),
                                     wo_v.at[pl.ds(p * STAGE_ROWS, STAGE_ROWS)],
                                     sem.at[ST0 + 2 * p + 1])

    def stage_step(j):
        if j - 1 < STAGE_PIECES:
            stage_in(j - 1).wait()
            stage_out(j - 1).start()
        if j + 1 < STAGE_PIECES:
            if j + 1 >= STAGE_SLOTS:
                stage_out(j + 1 - STAGE_SLOTS).wait()
            stage_in(j + 1).start()

    cp_x.start()
    cp_wq.start()
    stage_in(0).start()
    stage_in(1).start()
    cp_wuk.start()
    for b in range(B):
        for j in range(n_kv):
            kv_copy(b, j).start()
    cp_b1.start()
    cp_b2.start()
    cp_w1.start()
    cp_w2.start()
    cp_wuv.start()
    for cp in cp_wo:
        cp.start()

    e_v[...] = (lax.broadcasted_iota(jnp.int32, (LANES, W), 0)
                == lax.broadcasted_iota(jnp.int32, (LANES, W), 1) // HG
                ).astype(F32).astype(BF16)
    et_v[...] = (lax.broadcasted_iota(jnp.int32, (W, LANES), 0) // HG
                 == lax.broadcasted_iota(jnp.int32, (W, LANES), 1)
                 ).astype(F32).astype(BF16)

    def diag_mask(rows):
        return (lax.broadcasted_iota(jnp.int32, (rows, W), 0) % HG
                == lax.broadcasted_iota(jnp.int32, (rows, W), 1) % HG)

    def expand(a):
        st = jnp.concatenate([a[:, g * LANES:(g + 1) * LANES] for g in range(G)], axis=0)
        rep = jnp.dot(st, e_v[...], preferred_element_type=F32)
        return jnp.where(diag_mask(G * R), rep, 0.0).astype(BF16)

    def head_group(w_ref, g, hg):
        return w_ref[g * LANES:(g + 1) * LANES, hg * HG:(hg + 1) * HG, :].reshape(W, D)

    cp_x.wait()
    x32 = x_v[...].astype(F32)
    xs = [x32[b:b + 1] for b in range(B)]

    def rnd(a):
        return a.astype(BF16).astype(F32)

    xns = []
    for xb in xs:
        mu = jnp.mean(xb, axis=-1, keepdims=True)
        xc = xb - mu
        var = jnp.mean(xc * xc, axis=-1, keepdims=True)
        xns.append(rnd(xb - rnd(mu)) / rnd(jnp.sqrt(rnd(rnd(var) + 1e-5))))
    xrows = jnp.concatenate(
        [jnp.broadcast_to(xn, (HG, M)) for xn in xns], axis=0).astype(BF16)

    lq = expand(xrows)
    cp_wq.wait()
    stage_step(1)
    qs = []
    for hg in range(NHG):
        acc = jnp.zeros((R, D), F32)
        for g in range(G):
            acc += jnp.dot(lq[g * R:(g + 1) * R], head_group(wq_v, g, hg),
                           preferred_element_type=F32)
        qs.append(acc.astype(BF16))

    cp_wuk.wait()
    stage_step(2)
    dm = diag_mask(R)
    scale = rnd(jnp.full((1, 1), D ** -0.5, F32))
    for hg in range(NHG):
        for g in range(G):
            st = lax.dot_general(qs[hg], head_group(wuk_v, g, hg), NT,
                                 preferred_element_type=F32)
            k = hg * G + g
            lhs_v[k * R:(k + 1) * R, :] = jnp.where(dm, st * scale, 0.0).astype(BF16)
    qa = jnp.dot(lhs_v[...], et_v[...], preferred_element_type=F32).astype(BF16)
    for b in range(B):
        for hg in range(NHG):
            for g in range(G):
                r0 = (hg * G + g) * R + b * HG
                qa_v[b, hg * HG:(hg + 1) * HG, g * LANES:(g + 1) * LANES] = qa[r0:r0 + HG]

    m_v[...] = jnp.full(m_v.shape, -jnp.inf, F32)
    l_v[...] = jnp.zeros(l_v.shape, F32)
    acc_v[...] = jnp.zeros(acc_v.shape, F32)
    sub = KV_DMA_ROWS // TK

    def kv_step(t, carry):
        b = t // (S // TK)
        j = t % (S // TK)

        @pl.when(j % sub == 0)
        def _():
            kv_copy(b, j // sub).wait()

        for k in range(B * n_kv):
            pl.when(t == k * sub)(functools.partial(stage_step, 3 + k))

        c = ckv_v[b, pl.ds(pl.multiple_of(j * TK, TK), TK), :]
        s = lax.dot_general(qa_v[b], c, NT, preferred_element_type=F32)
        m_old = m_v[b]
        m_new = jnp.maximum(m_old, jnp.max(s, axis=-1, keepdims=True))
        alpha = jnp.exp(m_old - m_new)
        p = jnp.exp(s - m_new)
        l_v[b] = alpha * l_v[b] + jnp.sum(p, axis=-1, keepdims=True)
        acc_v[b] = alpha * acc_v[b] + jnp.dot(p.astype(BF16), c, preferred_element_type=F32)
        m_v[b] = m_new
        return carry

    lax.fori_loop(0, B * (S // TK), kv_step, 0)

    ctxc = [(acc_v[b] / l_v[b]).astype(BF16) for b in range(B)]
    for hg in range(NHG):
        a = jnp.concatenate([ctxc[b][hg * HG:(hg + 1) * HG] for b in range(B)], axis=0)
        lhs_v[hg * G * R:(hg + 1) * G * R, :] = expand(a)

    cp_b1.wait()
    cp_b2.wait()
    cp_w1.wait()
    hid = jnp.dot(xrows, w1_v[...], preferred_element_type=F32)
    hid = hid + b1_v[...].astype(F32).reshape(1, FF)
    hid = jax.nn.gelu(hid, approximate=True).astype(BF16)
    cp_w2.wait()
    y = jnp.dot(hid, w2_v[...], preferred_element_type=F32)
    y = y + b2_v[...].astype(F32).reshape(1, M)
    gate = y * jax.nn.sigmoid(y)
    even = lax.broadcasted_iota(jnp.int32, (SUB, M), 0) % 2 == 0
    fin_v[0] = jnp.where(even, gate[:SUB], gate[HG:HG + SUB])
    fin_v[1] = jnp.where(even, jnp.broadcast_to(xs[0], (SUB, M)),
                         jnp.broadcast_to(xs[1], (SUB, M)))
    for j in range(3 + B * n_kv, STAGE_PIECES + 1):
        stage_step(j)

    cp_wuv.wait()
    ctx = []
    for hg in range(NHG):
        acc = jnp.zeros((R, D), F32)
        for g in range(G):
            k = hg * G + g
            acc += jnp.dot(lhs_v[k * R:(k + 1) * R, :], head_group(wuv_v, g, hg),
                           preferred_element_type=F32)
        ctx.append(acc)

    row_i = lax.broadcasted_iota(jnp.int32, (R, D), 0) % HG
    lo = jnp.concatenate(
        [jnp.where(row_i == h % HG, ctx[h // HG], 0.0).astype(BF16)
         for h in range(H - vpu_heads)], axis=1)
    for b in range(B):
        for u in range(vpu_heads):
            i = b * HG + HG - vpu_heads + u
            row = ctx[NHG - 1][i:i + 1, :].astype(BF16).astype(F32)
            cb_v[b, u * D:(u + 1) * D] = jnp.transpose(jnp.broadcast_to(row, (LANES, D)))

    for p in range(max(STAGE_PIECES - STAGE_SLOTS, 0), STAGE_PIECES):
        stage_out(p).wait()
    r_staged = STAGE_PIECES * STAGE_ROWS
    s_v[...] = jnp.dot(lo[:, :r_staged], wo_v[:r_staged], preferred_element_type=F32)
    n_mxu = len(wo_splits) - n_vpu
    for k in range(n_mxu):
        r0, r1 = wo_splits[k]
        cp_wo[k].wait()
        part = s_v[...] + jnp.dot(lo[:, r0:r1], wo_v[r0:r1], preferred_element_type=F32)
        if k + 1 < n_mxu:
            s_v[...] = part
    for b in range(B):
        s_v[b * SUB:(b + 1) * SUB, :] = (part[b * HG:b * HG + SUB]
                                         + part[b * HG + SUB:(b + 1) * HG])
    v0 = (H - vpu_heads) * D
    for k in range(n_mxu, len(wo_splits)):
        r0, r1 = wo_splits[k]
        cp_wo[k].wait()
        accs = [s_v[b * SUB:(b + 1) * SUB, :] for b in range(B)]
        for r in range(r0, r1, HG):
            w32 = wo_v[r:r + HG].astype(F32)
            for b in range(B):
                cb = cb_v[b, r - v0:r - v0 + HG, :]
                prod = w32 * jnp.concatenate([cb] * (M // LANES), axis=1)
                accs[b] = accs[b] + prod[:SUB] + prod[SUB:]
        if k + 1 < len(wo_splits):
            for b in range(B):
                s_v[b * SUB:(b + 1) * SUB, :] = accs[b]
    u = (jnp.where(even, accs[0], accs[1])
         + pltpu.roll(jnp.where(even, accs[1], accs[0]), SUB - 1, axis=0))
    u = u + pltpu.roll(u, 2, axis=0)
    u = u + pltpu.roll(u, 4, axis=0)
    o_ref[...] = (fin_v[1] + u * fin_v[0])[:B].astype(o_ref.dtype)


def _compiler_params():
    vmem = 100 * 1024 * 1024
    try:
        return pltpu.CompilerParams(vmem_limit_bytes=vmem, disable_semaphore_checks=True)
    except TypeError:
        return pltpu.CompilerParams(vmem_limit_bytes=vmem)


@jax.jit
def pallas_recurrent_scan__compressed_kv_cla__dense_activation_gelu__decode_kernel(
    A_x: jax.Array,
    A_c_kv: jax.Array,
    A_w_q: jax.Array,
    A_w_uk: jax.Array,
    A_w_uv: jax.Array,
    A_w_o: jax.Array,
    B_x: jax.Array,
    B_w1: jax.Array,
    B_b1: jax.Array,
    B_w2: jax.Array,
    B_b2: jax.Array,
):
    del B_x
    B, Sq, M = A_x.shape
    _, S, C = A_c_kv.shape
    _, H, D = A_w_q.shape
    FF = B_w1.shape[1]
    assert B == 2 and Sq == 1 and M == C and D == LANES and H % HG == 0 and S % KV_DMA_ROWS == 0
    assert sum(WO_VPU_TAIL) % D == 0 and sum(WO_VPU_TAIL) <= HG * D
    G = C // LANES
    R = B * HG
    W = LANES * HG

    r = STAGE_PIECES * STAGE_ROWS
    sizes = (H * D - r - sum(WO_MXU_TAIL) - sum(WO_VPU_TAIL),) + WO_MXU_TAIL + WO_VPU_TAIL
    wo_splits = []
    for n in sizes:
        wo_splits.append((r, r + n))
        r += n
    n_sem = 8 + len(wo_splits) + B * (S // KV_DMA_ROWS) + 2 * STAGE_PIECES

    kernel = functools.partial(_kernel, B=B, S=S, C=C, H=H, D=D, M=M, FF=FF,
                               wo_splits=tuple(wo_splits))
    hbm = pl.BlockSpec(memory_space=pl.ANY)
    out = pl.pallas_call(
        kernel,
        out_shape=jax.ShapeDtypeStruct((B, M), A_x.dtype),
        in_specs=[hbm] * 10,
        out_specs=pl.BlockSpec(memory_space=pltpu.VMEM),
        scratch_shapes=[
            pltpu.VMEM((B, M), BF16),
            pltpu.VMEM(A_c_kv.shape, BF16),
            pltpu.VMEM(A_w_q.shape, BF16),
            pltpu.VMEM(A_w_uk.shape, BF16),
            pltpu.VMEM(A_w_uv.shape, BF16),
            pltpu.VMEM((H * D, M), BF16),
            pltpu.VMEM(B_w1.shape, BF16),
            pltpu.VMEM(B_b1.shape, BF16),
            pltpu.VMEM(B_w2.shape, BF16),
            pltpu.VMEM(B_b2.shape, BF16),
            pltpu.VMEM((LANES, W), BF16),
            pltpu.VMEM((W, LANES), BF16),
            pltpu.VMEM(((H // HG) * G * R, W), BF16),
            pltpu.VMEM((B, H, C), BF16),
            pltpu.VMEM((B, H, 1), F32),
            pltpu.VMEM((B, H, 1), F32),
            pltpu.VMEM((B, H, C), F32),
            pltpu.VMEM((R, M), F32),
            pltpu.VMEM((2, SUB, M), F32),
            pltpu.VMEM((B, sum(WO_VPU_TAIL), LANES), F32),
            pltpu.SMEM((STAGE_SLOTS * STAGE_ROWS, M), BF16),
            pltpu.SemaphoreType.DMA((n_sem,)),
        ],
        compiler_params=_compiler_params(),
    )(A_x.reshape(B, M), A_c_kv, A_w_q, A_w_uk, A_w_uv, A_w_o.reshape(H * D, M),
      B_w1, B_b1, B_w2, B_b2)
    return out.reshape(B, Sq, M)
```
